```python
import os as _os
_os.environ.setdefault("JAX_PLATFORMS", "cpu")
import jax
import jax.numpy as jnp

def _softmax(x, axis=-1):
    return jax.nn.softmax(x, axis=axis)
def _gelu(x):
    return jax.nn.gelu(x, approximate=True)
def _silu(x):
    return jax.nn.silu(x)
def _sigmoid(x):
    return jax.nn.sigmoid(x)
def _layernorm(x, axis=-1, eps=1e-5):
    m = jnp.mean(x, axis=axis, keepdims=True)
    v = jnp.var(x, axis=axis, keepdims=True)
    return (x - m) / jnp.sqrt(v + eps)
def _scatter_add(tgt, idx, src, axis=0):
    return tgt.at[idx].add(src)
def _segment_sum(src, seg, n):
    return jax.ops.segment_sum(src, seg, n)
class _Rng:
    def __init__(self, key):
        self._k = key
    def _next(self):
        self._k, sub = jax.random.split(self._k)
        return sub
    def normal(self, shape):
        return jax.random.normal(self._next(), shape, dtype=jnp.bfloat16)
    def randint(self, lo, hi, shape):
        return jax.random.randint(self._next(), shape, lo, hi, dtype=jnp.int32)
    def uniform(self, shape, lo=0.0, hi=1.0):
        return jax.random.uniform(self._next(), shape, jnp.bfloat16, lo, hi)
    def permutation(self, n):
        return jax.random.permutation(self._next(), n)


kernel_name = 'concat_heads__mha_block_cached__gqa_block_cached__near_ridge'

def setup_inputs():
    _rng = _Rng(jax.random.key(int.from_bytes(__import__("os").urandom(4), "little")))
    _w = (lambda a: (lambda t: t.astype(jnp.bfloat16) if jnp.issubdtype(t.dtype, jnp.floating) else t)(jnp.asarray(a)))
    def _A_setup():
        B, Sq, D = 8, 128, 640
        H, Sk, Dh = 32, 1024, 192
        return {
            "x": _w((lambda *s: _rng.normal(s) * 0.8)(B, Sq, D)),
            "k_cache": _w((lambda *s: _rng.normal(s) * 0.8)(B, H, Sk, Dh)),
            "v_cache": _w((lambda *s: _rng.normal(s) * 0.05)(B, H, Sk, Dh)),
            "wq": _w((lambda *s: _rng.normal(s) * 0.8)(D, H * Dh) * (D ** -0.5)),
            "wo": _w((lambda *s: _rng.normal(s) * 0.05)(H * Dh, D) * ((H * Dh) ** -0.5)),
        }
    _A_in = _A_setup()

    def _B_setup():
        B, Sq, D = 8, 128, 640
        Hq, Hkv, Sk, Dh = 32, 32, 1024, 192
        assert Hq % Hkv == 0, (Hq, Hkv)
        return {
            "x": _w((lambda *s: _rng.normal(s) * 0.8)(B, Sq, D)),
            "k_cache": _w((lambda *s: _rng.normal(s) * 0.8)(B, Hkv, Sk, Dh)),
            "v_cache": _w((lambda *s: _rng.normal(s) * 0.05)(B, Hkv, Sk, Dh)),
            "wq": _w((lambda *s: _rng.normal(s) * 0.8)(D, Hq * Dh) * (D ** -0.5)),
            "wo": _w((lambda *s: _rng.normal(s) * 0.05)(Hq * Dh, D) * ((Hq * Dh) ** -0.5)),
        }
    _B_in = _B_setup()

    return {
        "A_x": _A_in["x"],
        "A_k_cache": _A_in["k_cache"],
        "A_v_cache": _A_in["v_cache"],
        "A_wq": _A_in["wq"],
        "A_wo": _A_in["wo"],
        "B_x": _B_in["x"],
        "B_k_cache": _B_in["k_cache"],
        "B_v_cache": _B_in["v_cache"],
        "B_wq": _B_in["wq"],
        "B_wo": _B_in["wo"],
    }

def reference(A_x, A_k_cache, A_v_cache, A_wq, A_wo, B_x, B_k_cache, B_v_cache, B_wq, B_wo):
    def _A_ref(x, k_cache, v_cache, wq, wo):
        B, Sq, D = x.shape
        H, Dh = 32, 192
        q = (lambda x, *d: x.transpose(*d))((x @ wq).reshape(B, Sq, H, Dh), 0, 2, 1, 3)
        scores = jnp.einsum("bhqd,bhkd->bhqk", q, k_cache) * (Dh ** -0.5)
        p = _softmax(scores, axis=-1)
        o = jnp.einsum("bhqk,bhkd->bhqd", p, v_cache)
        return (lambda x, *d: x.transpose(*d))(o, 0, 2, 1, 3).reshape(B, Sq, H * Dh) @ wo

    def _B_ref(x, k_cache, v_cache, wq, wo):
        B, Sq, D = x.shape
        Hq, Dh = 32, 192
        Hkv = k_cache.shape[1]
        rep = Hq // Hkv
        q = (lambda x, *d: x.transpose(*d))((x @ wq).reshape(B, Sq, Hq, Dh), 0, 2, 1, 3)
        k = jnp.repeat(k_cache, rep, axis=1)
        v = jnp.repeat(v_cache, rep, axis=1)
        scores = jnp.einsum("bhqd,bhkd->bhqk", q, k) * (Dh ** -0.5)
        p = _softmax(scores, axis=-1)
        o = jnp.einsum("bhqk,bhkd->bhqd", p, v)
        return (lambda x, *d: x.transpose(*d))(o, 0, 2, 1, 3).reshape(B, Sq, Hq * Dh) @ wo

    a = _A_ref(A_x, A_k_cache, A_v_cache, A_wq, A_wo)
    b = _B_ref(B_x, B_k_cache, B_v_cache, B_wq, B_wo)
    return jnp.concatenate([a, b], axis=-1)
```

```python
import functools
import math
import jax
import jax.numpy as jnp
from jax import lax
import jax.experimental.pallas as pl
import jax.experimental.pallas.tpu as pltpu

B, SQ, D, H, SK, DH = 8, 128, 640, 32, 1024, 192
NP = H // 2
PW = 2 * DH
QSCALE = (DH ** -0.5) * math.log2(math.e)
NSTEP = NP * B


def _qk(q, kt_ref, h):
    kt = kt_ref[pl.ds(h * 128, 256), :]
    return jnp.dot(q, kt, preferred_element_type=jnp.float32)


def _softmax(s):
    m = jnp.max(s, axis=-1, keepdims=True)
    p = jnp.exp2(s - m)
    l = jnp.sum(p, axis=-1, keepdims=True)
    return p.astype(jnp.bfloat16), l


def _pv(p, vt_ref, h):
    vt = vt_ref[pl.ds(h * DH, DH), :]
    return lax.dot_general(vt, p, (((1,), (1,)), ((), ())),
                           preferred_element_type=jnp.float32)


def _finish(ot0, ot1, l0, l1):
    o = jnp.concatenate([ot0, ot1], axis=0).T
    lane = lax.broadcasted_iota(jnp.int32, (SQ, PW), 1)
    inv = jnp.where(lane < DH, 1.0 / l0, 1.0 / l1)
    return (o * inv).astype(jnp.bfloat16)


def _qproj(x_ref, wq_ref, row, q_sc, br):
    lane = lax.broadcasted_iota(jnp.int32, (SQ, 256), 1)
    q = jnp.dot(x_ref[pl.ds(row, SQ), :], wq_ref[...], preferred_element_type=jnp.float32) * QSCALE
    q_sc[br, 0] = jnp.where(lane < DH, q[:, 0:256], 0.0).astype(jnp.bfloat16)
    q_sc[br, 1] = jnp.where(lane >= 64, q[:, 128:384], 0.0).astype(jnp.bfloat16)


def _kernel(xa_ref, wqa_ref, kta_ref, vta_ref, woa_ref,
            xb_ref, wqb_ref, ktb_ref, vtb_ref, wob_ref,
            out_ref, q_sc, acc_sc):
    g = pl.program_id(0)
    b = pl.program_id(1)

    @pl.when((g == 0) & (b == 0))
    def _():
        _qproj(xa_ref, wqa_ref, 0, q_sc, 0)
        _qproj(xb_ref, wqb_ref, 0, q_sc, 1)
        acc_sc[...] = jnp.zeros_like(acc_sc)

    row = pl.multiple_of(b * SQ, SQ)
    row_next = pl.multiple_of(((b + 1) % B) * SQ, SQ)

    qa0 = q_sc[0, 0]
    qa1 = q_sc[0, 1]
    qb0 = q_sc[1, 0]
    qb1 = q_sc[1, 1]

    sa0 = _qk(qa0, kta_ref, 0)
    sa1 = _qk(qa1, kta_ref, 1)
    pa0, la0 = _softmax(sa0)
    oa0 = _pv(pa0, vta_ref, 0)
    sb0 = _qk(qb0, ktb_ref, 0)
    pa1, la1 = _softmax(sa1)
    oa1 = _pv(pa1, vta_ref, 1)
    sb1 = _qk(qb1, ktb_ref, 1)
    pb0, lb0 = _softmax(sb0)
    ob0 = _pv(pb0, vtb_ref, 0)
    _qproj(xa_ref, wqa_ref, row_next, q_sc, 0)
    pb1, lb1 = _softmax(sb1)
    ob1 = _pv(pb1, vtb_ref, 1)
    _qproj(xb_ref, wqb_ref, row_next, q_sc, 1)
    oa = _finish(oa0, oa1, la0, la1)
    acc_sc[0, pl.ds(row, SQ), :] += jnp.dot(oa, woa_ref[...], preferred_element_type=jnp.float32)
    ob = _finish(ob0, ob1, lb0, lb1)
    acc_sc[1, pl.ds(row, SQ), :] += jnp.dot(ob, wob_ref[...], preferred_element_type=jnp.float32)

    @pl.when(g == NP - 1)
    def _():
        out_ref[:, 0:D] = acc_sc[0, pl.ds(row, SQ), :].astype(out_ref.dtype)
        out_ref[:, D:2 * D] = acc_sc[1, pl.ds(row, SQ), :].astype(out_ref.dtype)


@jax.jit
def pallas_concat_heads__mha_block_cached__gqa_block_cached__near_ridge_kernel(
    A_x, A_k_cache, A_v_cache, A_wq, A_wo, B_x, B_k_cache, B_v_cache, B_wq, B_wo):
    def prep_kv(a):
        return jnp.swapaxes(a, 2, 3).reshape(B, NP, PW, SK)

    x_spec = pl.BlockSpec((B * SQ, D), lambda g, b: (0, 0))
    wq_spec = pl.BlockSpec((D, PW), lambda g, b: (0, jnp.minimum((g * B + b + 1) // B, NP - 1)))
    kv_spec = pl.BlockSpec((None, None, PW, SK), lambda g, b: (b, g, 0, 0))
    wo_spec = pl.BlockSpec((PW, D), lambda g, b: (g, 0))
    specs = [x_spec, wq_spec, kv_spec, kv_spec, wo_spec]
    out = pl.pallas_call(
        _kernel,
        grid=(NP, B),
        in_specs=specs + specs,
        out_specs=pl.BlockSpec((SQ, 2 * D), lambda g, b: (jnp.where(g == NP - 1, b, 0), 0)),
        out_shape=jax.ShapeDtypeStruct((B * SQ, 2 * D), jnp.bfloat16),
        scratch_shapes=[
            pltpu.VMEM((2, 2, SQ, 256), jnp.bfloat16),
            pltpu.VMEM((2, B * SQ, D), jnp.float32),
        ],
        compiler_params=pltpu.CompilerParams(
            dimension_semantics=("arbitrary", "arbitrary"),
            vmem_limit_bytes=100 * 1024 * 1024,
        ),
    )(A_x.reshape(B * SQ, D), A_wq, prep_kv(A_k_cache), prep_kv(A_v_cache), A_wo,
      B_x.reshape(B * SQ, D), B_wq, prep_kv(B_k_cache), prep_kv(B_v_cache), B_wo)
    return out.reshape(B, SQ, 2 * D)
```

```python
import math
import jax
import jax.numpy as jnp
from jax import lax
import jax.experimental.pallas as pl
import jax.experimental.pallas.tpu as pltpu

B, SQ, D, H, SK, DH = 8, 128, 640, 32, 1024, 192
NP = H // 2
PW = 2 * DH
QSCALE = (DH ** -0.5) * math.log2(math.e)
NSTEP = NP * B
NBUF = 4
CH = 16
NSPLIT = 3
KV_PLAN = [(j, h * (PW // NSPLIT) + c * CH)
           for c in range(PW // NSPLIT // CH) for j in range(4) for h in range(NSPLIT)]
NKV = len(KV_PLAN)
AHEAD = 144
NPT = 8
PER_PT = NKV // NPT
WQ_CH = D // 16
WO_CH = PW // 16
W_LEAD = 11
X_CH = 32


def _qk(q, kt_ref, h):
    kt = kt_ref[pl.ds(h * 128, 256), :]
    return jnp.dot(q, kt, preferred_element_type=jnp.float32)


def _softmax(s):
    m = jnp.max(s, axis=-1, keepdims=True)
    p = jnp.exp2(s - m)
    l = jnp.sum(p, axis=-1, keepdims=True)
    return p.astype(jnp.bfloat16), l


def _pv(p, vt_ref, h):
    vt = vt_ref[pl.ds(h * DH, DH), :]
    return lax.dot_general(vt, p, (((1,), (1,)), ((), ())),
                           preferred_element_type=jnp.float32)


def _finish(ot0, ot1, l0, l1):
    o = jnp.concatenate([ot0, ot1], axis=0).T
    lane = lax.broadcasted_iota(jnp.int32, (SQ, PW), 1)
    inv = jnp.where(lane < DH, 1.0 / l0, 1.0 / l1)
    return (o * inv).astype(jnp.bfloat16)


def _qproj(x_ref, wq_ref, row, q_sc, br):
    lane = lax.broadcasted_iota(jnp.int32, (SQ, 256), 1)
    q = jnp.dot(x_ref[pl.ds(row, SQ), :], wq_ref[...], preferred_element_type=jnp.float32) * QSCALE
    q_sc[br, 0] = jnp.where(lane < DH, q[:, 0:256], 0.0).astype(jnp.bfloat16)
    q_sc[br, 1] = jnp.where(lane >= 64, q[:, 128:384], 0.0).astype(jnp.bfloat16)


def _mult(v, n):
    return v if isinstance(v, int) else pl.multiple_of(v, n)


def _kernel(xa_hbm, wqa_hbm, ka_hbm, va_hbm, woa_hbm,
            xb_hbm, wqb_hbm, kb_hbm, vb_hbm, wob_hbm,
            out_hbm,
            x_buf, wq_buf, wo_buf, kv_buf, q_sc, acc_sc, out_buf,
            sem_x, sem_wq, sem_wo, sem_kv, sem_out):
    x_hbm = (xa_hbm, xb_hbm)
    wq_hbm = (wqa_hbm, wqb_hbm)
    wo_hbm = (woa_hbm, wob_hbm)
    kv_hbm = (ka_hbm, va_hbm, kb_hbm, vb_hbm)

    def x_start(c, br, prio):
        rows = pl.ds(c * X_CH, X_CH)
        sem = sem_x.at[0] if c * X_CH < SQ else sem_x.at[1]
        pltpu.make_async_copy(x_hbm[br].at[rows, :], x_buf.at[br, rows, :], sem).start(priority=prio)

    def x_wait(i):
        rows = pl.ds(0, SQ) if i == 0 else pl.ds(SQ, (B - 1) * SQ)
        ref = x_buf.at[:, rows, :]
        pltpu.make_async_copy(ref, ref, sem_x.at[i]).wait()

    def wq_start(g, piece, br, prio):
        rows = pl.ds(_mult(piece * WQ_CH, 8), WQ_CH)
        pltpu.make_async_copy(wq_hbm[br].at[rows, pl.ds(_mult(g * PW, 128), PW)],
                              wq_buf.at[g, br, rows, :], sem_wq.at[g % 2]).start(priority=prio)

    def wo_start(g, piece, br, prio):
        pltpu.make_async_copy(wo_hbm[br].at[pl.ds(_mult(g * PW + piece * WO_CH, 8), WO_CH), :],
                              wo_buf.at[g, br, pl.ds(_mult(piece * WO_CH, 8), WO_CH), :],
                              sem_wo.at[g % 2]).start(priority=prio)

    def wq_wait(g):
        pltpu.make_async_copy(wq_buf.at[g], wq_buf.at[g], sem_wq.at[g % 2]).wait()

    def wo_wait(g):
        pltpu.make_async_copy(wo_buf.at[g], wo_buf.at[g], sem_wo.at[g % 2]).wait()

    def w_start(g, i, k):
        piece = 2 * i + (k // 4)
        br = k % 2
        if (k // 2) % 2 == 0:
            wq_start(g, piece, br, k % 2)
        else:
            wo_start(g, piece, br, k % 2)

    def kv_start(s, lo, hi):
        slot = s % NBUF
        bb = s % B
        gg = s // B
        for k in range(lo, hi):
            j, off = KV_PLAN[k]
            pltpu.make_async_copy(kv_hbm[j].at[bb, gg, pl.ds(off, CH), :],
                                  kv_buf.at[slot, j, pl.ds(off, CH), :],
                                  sem_kv.at[slot]).start(priority=k % 2)

    def kv_wait(s):
        slot = s % NBUF
        pltpu.make_async_copy(kv_buf.at[slot], kv_buf.at[slot], sem_kv.at[slot]).wait()

    def out_copy(i):
        rows = pl.ds(0, (B - 1) * SQ) if i == 0 else pl.ds((B - 1) * SQ, SQ)
        return pltpu.make_async_copy(out_buf.at[rows, :], out_hbm.at[rows, :], sem_out.at[i])

    for piece in range(16):
        for br in range(2):
            wq_start(0, piece, br, br)
    for c in range(SQ // X_CH):
        for br in range(2):
            x_start(c, br, br)
    kv_start(0, 0, 40)
    acc_sc[...] = jnp.zeros_like(acc_sc)
    kv_start(0, 40, NKV)
    wq_wait(0)
    x_wait(0)
    for br in range(2):
        _qproj(x_buf.at[br], wq_buf.at[0, br], 0, q_sc, br)
    for piece in range(16):
        for br in range(2):
            wo_start(0, piece, br, br)
    for c in range(SQ // X_CH, B * SQ // X_CH):
        for br in range(2):
            x_start(c, br, br)
    for i in range(W_LEAD - B):
        for k in range(8):
            w_start(1, i, k)
    kv_start(1, 0, AHEAD - NKV)
    wo_wait(0)
    x_wait(1)

    def step(s, carry):
        g = s // B
        b = s % B
        gw = (s + W_LEAD) // B
        iw = (s + W_LEAD) % B

        def issue(pt):
            lo = AHEAD + pt * PER_PT
            ds_, lo = lo // NKV, lo % NKV
            if ds_ == 1:
                kv_start(s + 1, lo, lo + PER_PT)
            else:
                for k in range(lo, lo + PER_PT, 2):
                    @pl.when(s + ds_ < NSTEP)
                    def _():
                        kv_start(s + ds_, k, k + 2)

            @pl.when(gw < NP)
            def _():
                w_start(gw, iw, pt)

        @pl.when(b == B - 1)
        def _():
            wq_wait(g + 1)
            wo_wait(g + 1)

        kv_wait(s)

        slot = s % NBUF
        kta_ref = kv_buf.at[slot, 0]
        vta_ref = kv_buf.at[slot, 1]
        ktb_ref = kv_buf.at[slot, 2]
        vtb_ref = kv_buf.at[slot, 3]
        gq = (s + 1) // B
        row = pl.multiple_of(b * SQ, SQ)
        row_next = pl.multiple_of(((b + 1) % B) * SQ, SQ)

        qa0 = q_sc[0, 0]
        qa1 = q_sc[0, 1]
        qb0 = q_sc[1, 0]
        qb1 = q_sc[1, 1]

        issue(0)
        sa0 = _qk(qa0, kta_ref, 0)
        sa1 = _qk(qa1, kta_ref, 1)
        issue(1)
        pa0, la0 = _softmax(sa0)
        oa0 = _pv(pa0, vta_ref, 0)
        issue(2)
        sb0 = _qk(qb0, ktb_ref, 0)
        pa1, la1 = _softmax(sa1)
        oa1 = _pv(pa1, vta_ref, 1)
        issue(3)
        sb1 = _qk(qb1, ktb_ref, 1)
        issue(4)
        pb0, lb0 = _softmax(sb0)
        ob0 = _pv(pb0, vtb_ref, 0)
        _qproj(x_buf.at[0], wq_buf.at[gq, 0], row_next, q_sc, 0)
        issue(5)
        pb1, lb1 = _softmax(sb1)
        ob1 = _pv(pb1, vtb_ref, 1)
        issue(6)
        _qproj(x_buf.at[1], wq_buf.at[gq, 1], row_next, q_sc, 1)
        oa = _finish(oa0, oa1, la0, la1)
        acc_sc[0, pl.ds(row, SQ), :] += jnp.dot(oa, wo_buf[g, 0], preferred_element_type=jnp.float32)
        issue(7)
        ob = _finish(ob0, ob1, lb0, lb1)
        acc_sc[1, pl.ds(row, SQ), :] += jnp.dot(ob, wo_buf[g, 1], preferred_element_type=jnp.float32)

        @pl.when(g == NP - 1)
        def _():
            out_buf[pl.ds(row, SQ), 0:D] = acc_sc[0, pl.ds(row, SQ), :].astype(out_buf.dtype)
            out_buf[pl.ds(row, SQ), D:2 * D] = acc_sc[1, pl.ds(row, SQ), :].astype(out_buf.dtype)

        return carry

    lax.fori_loop(0, NSTEP - 1, step, 0)

    s = NSTEP - 1
    slot = s % NBUF
    rows = pl.ds((B - 1) * SQ, SQ)
    kv_wait(s)
    out_copy(0).start()
    kta_ref = kv_buf.at[slot, 0]
    vta_ref = kv_buf.at[slot, 1]
    ktb_ref = kv_buf.at[slot, 2]
    vtb_ref = kv_buf.at[slot, 3]
    sa0 = _qk(q_sc[0, 0], kta_ref, 0)
    sa1 = _qk(q_sc[0, 1], kta_ref, 1)
    pa0, la0 = _softmax(sa0)
    oa0 = _pv(pa0, vta_ref, 0)
    sb0 = _qk(q_sc[1, 0], ktb_ref, 0)
    pa1, la1 = _softmax(sa1)
    oa1 = _pv(pa1, vta_ref, 1)
    sb1 = _qk(q_sc[1, 1], ktb_ref, 1)
    pb0, lb0 = _softmax(sb0)
    ob0 = _pv(pb0, vtb_ref, 0)
    oa = _finish(oa0, oa1, la0, la1)
    ya = acc_sc[0, rows, :] + jnp.dot(oa, wo_buf[NP - 1, 0], preferred_element_type=jnp.float32)
    out_buf[rows, 0:D] = ya.astype(out_buf.dtype)
    pb1, lb1 = _softmax(sb1)
    ob1 = _pv(pb1, vtb_ref, 1)
    ob = _finish(ob0, ob1, lb0, lb1)
    yb = acc_sc[1, rows, :] + jnp.dot(ob, wo_buf[NP - 1, 1], preferred_element_type=jnp.float32)
    out_buf[rows, D:2 * D] = yb.astype(out_buf.dtype)
    out_copy(1).start()
    out_copy(0).wait()
    out_copy(1).wait()


@jax.jit
def pallas_concat_heads__mha_block_cached__gqa_block_cached__near_ridge_kernel(
    A_x, A_k_cache, A_v_cache, A_wq, A_wo, B_x, B_k_cache, B_v_cache, B_wq, B_wo):
    def prep_kv(a):
        return jnp.swapaxes(a, 2, 3).reshape(B, NP, PW, SK)

    any_spec = pl.BlockSpec(memory_space=pl.ANY)
    out = pl.pallas_call(
        _kernel,
        in_specs=[any_spec] * 10,
        out_specs=any_spec,
        out_shape=jax.ShapeDtypeStruct((B * SQ, 2 * D), jnp.bfloat16),
        scratch_shapes=[
            pltpu.VMEM((2, B * SQ, D), jnp.bfloat16),
            pltpu.VMEM((NP, 2, D, PW), jnp.bfloat16),
            pltpu.VMEM((NP, 2, PW, D), jnp.bfloat16),
            pltpu.VMEM((NBUF, 4, PW, SK), jnp.bfloat16),
            pltpu.VMEM((2, 2, SQ, 256), jnp.bfloat16),
            pltpu.VMEM((2, B * SQ, D), jnp.float32),
            pltpu.VMEM((B * SQ, 2 * D), jnp.bfloat16),
            pltpu.SemaphoreType.DMA((2,)),
            pltpu.SemaphoreType.DMA((2,)),
            pltpu.SemaphoreType.DMA((2,)),
            pltpu.SemaphoreType.DMA((NBUF,)),
            pltpu.SemaphoreType.DMA((2,)),
        ],
        compiler_params=pltpu.CompilerParams(
            vmem_limit_bytes=100 * 1024 * 1024,
            disable_bounds_checks=True,
        ),
    )(A_x.reshape(B * SQ, D), A_wq, prep_kv(A_k_cache), prep_kv(A_v_cache), A_wo,
      B_x.reshape(B * SQ, D), B_wq, prep_kv(B_k_cache), prep_kv(B_v_cache), B_wo)
    return out.reshape(B, SQ, 2 * D)
```

```python
import math
import jax
import jax.numpy as jnp
from jax import lax
import jax.experimental.pallas as pl
import jax.experimental.pallas.tpu as pltpu

B, SQ, D, H, SK, DH = 8, 128, 640, 32, 1024, 192
NP = H // 2
PW = 2 * DH
QSCALE = (DH ** -0.5) * math.log2(math.e)
NU = NP * B
CFG = dict(NBUF=4, SHIFT=13, MARGIN=96, W_LEAD=12, OUT_CH=16, COMPUTE=3, ORDER=3)
NBUF = CFG['NBUF']; SHIFT = CFG['SHIFT']; MARGIN = CFG['MARGIN']
W_LEAD = CFG['W_LEAD']; OUT_CH = CFG['OUT_CH']; COMPUTE = CFG['COMPUTE']

BLK = 16
CT = SK // 128
HT = DH // 8 * CT
DT = D // 128
XT = SQ // 8 * DT
WOT = PW // 8 * DT


def _cuts(ntiles, n):
    inner = [SHIFT + BLK * k for k in range(ntiles // BLK) if 0 < SHIFT + BLK * k < ntiles]
    while len(inner) > n - 1:
        inner = inner[:-1] if SHIFT >= BLK // 2 else inner[1:]
    return [0] + inner + [ntiles]


NCH = HT // BLK
_KC = _cuts(HT, NCH)
ROUND = [(d, j, _KC[c], _KC[c + 1] - _KC[c])
         for c in range(NCH) for d in range(2) for j in range(4)]
NKV = len(ROUND)
NPT = 12
PER_PT = NKV // NPT
WQ_CH = D // 16
_XC = _cuts(XT, XT // BLK)

SLOT_T = 4 * 2 * HT
X_BASE = NBUF * SLOT_T
WO_BASE = X_BASE + B * 2 * XT
U_TILES = WO_BASE + NP * 2 * WOT


def _slab(u_ref, t0, nrows, ct):
    n = nrows // 8
    v = u_ref[pl.ds(t0, n * ct)].reshape(n, ct, 8, 128)
    return jnp.concatenate([v[:, c].reshape(nrows, 128) for c in range(ct)], axis=1)


def _softmax(s):
    m = jnp.max(s, axis=-1, keepdims=True)
    p = jnp.exp2(s - m)
    l = jnp.sum(p, axis=-1, keepdims=True)
    return p.astype(jnp.bfloat16), l


def _finish(ot0, ot1, l0, l1):
    o = jnp.concatenate([ot0, ot1], axis=0).T
    lane = lax.broadcasted_iota(jnp.int32, (SQ, PW), 1)
    inv = jnp.where(lane < DH, 1.0 / l0, 1.0 / l1)
    return (o * inv).astype(jnp.bfloat16)


def _div(v, n):
    return v // n if isinstance(v, int) else lax.shift_right_logical(v, n.bit_length() - 1)


def _mod(v, n):
    return v % n if isinstance(v, int) else v & (n - 1)


def _mult(v, n):
    return v if isinstance(v, int) else pl.multiple_of(v, n)


def _kernel(xa_hbm, wqa_hbm, ka_hbm, va_hbm, woa_hbm,
            xb_hbm, wqb_hbm, kb_hbm, vb_hbm, wob_hbm,
            out_hbm,
            u_buf, wq_buf, q_sc, o0_sc, l0_sc, acc_sc, out_buf,
            sem_x, sem_wq, sem_wo, sem_kv, sem_out):
    x_hbm = (xa_hbm, xb_hbm)
    wq_hbm = (wqa_hbm, wqb_hbm)
    wo_hbm = (woa_hbm, wob_hbm)
    kv_hbm = (ka_hbm, va_hbm, kb_hbm, vb_hbm)

    def u_wait(t0, nt, sem):
        ref = u_buf.at[pl.ds(t0, nt)]
        pltpu.make_async_copy(ref, ref, sem).wait()

    def x_start(b):
        for c in range(len(_XC) - 1):
            for br in range(2):
                t0, nt = _XC[c], _XC[c + 1] - _XC[c]
                pltpu.make_async_copy(x_hbm[br].at[pl.ds(b * XT + t0, nt)],
                                      u_buf.at[pl.ds(X_BASE + (2 * b + br) * XT + t0, nt)],
                                      sem_x.at[0 if b < 2 else 1]).start(priority=br)

    def x_wait(i):
        if i == 0:
            u_wait(X_BASE, 4 * XT, sem_x.at[0])
        else:
            u_wait(X_BASE + 4 * XT, 2 * (B - 2) * XT, sem_x.at[1])

    def wq_start(g, piece, br):
        rows = pl.ds(_mult(piece * WQ_CH, 8), WQ_CH)
        pltpu.make_async_copy(wq_hbm[br].at[rows, pl.ds(_mult(g * PW, 128), PW)],
                              wq_buf.at[g, br, rows, :], sem_wq.at[_mod(g, 2)]).start(priority=br)

    def wo_start(g, piece, br):
        t0 = piece * (WOT // 16)
        pltpu.make_async_copy(wo_hbm[br].at[pl.ds(g * WOT + t0, WOT // 16)],
                              u_buf.at[pl.ds(WO_BASE + (2 * g + br) * WOT + t0, WOT // 16)],
                              sem_wo.at[_mod(g, 2)]).start(priority=br)

    def wq_wait(g):
        pltpu.make_async_copy(wq_buf.at[g], wq_buf.at[g], sem_wq.at[_mod(g, 2)]).wait()

    def wo_wait(g):
        u_wait(WO_BASE + 2 * g * WOT, 2 * WOT, sem_wo.at[_mod(g, 2)])

    def w_pair_start(g, i, k):
        piece = 2 * i + (k // 2)
        for br in range(2):
            if k % 2 == 0:
                wq_start(g, piece, br)
            else:
                wo_start(g, piece, br)

    def slot_of(r):
        return _mod(r + 1, NBUF)

    def kv_base(r, j):
        return slot_of(r) * SLOT_T + j * 2 * HT

    def kv_one(r, k):
        d, j, t0, nt = ROUND[k]
        u = r + d
        h = 1 - d
        pltpu.make_async_copy(kv_hbm[j].at[_mod(u, B), 2 * _div(u, B) + h, pl.ds(t0, nt)],
                              u_buf.at[pl.ds(kv_base(r, j) + h * HT + t0, nt)],
                              sem_kv.at[slot_of(r)]).start(priority=k % 2)

    def kv_static(r, lo, hi):
        for k in range(lo, hi):
            if 0 <= r + ROUND[k][0] < NU:
                kv_one(r, k)

    def kv_wait(r, h=None):
        if h is None:
            u_wait(kv_base(r, 0), SLOT_T, sem_kv.at[slot_of(r)])
        else:
            for j in range(4):
                u_wait(kv_base(r, j) + h * HT, HT, sem_kv.at[slot_of(r)])

    OUT_PARTS = ((0, (B - 2) * SQ, 6), ((B - 2) * SQ, SQ, 4), ((B - 1) * SQ, SQ, 4))

    def out_start(i):
        lo, nrows, ns = OUT_PARTS[i]
        n = nrows // OUT_CH
        for k in range(n):
            c = (k % ns) * (n // ns) + k // ns
            rows = pl.ds(lo + c * OUT_CH, OUT_CH)
            pltpu.make_async_copy(out_buf.at[rows, :], out_hbm.at[rows, :],
                                  sem_out.at[i]).start(priority=k % 2)

    def out_wait(i):
        rows = pl.ds(OUT_PARTS[i][0], OUT_PARTS[i][1])
        pltpu.make_async_copy(out_buf.at[rows, :], out_buf.at[rows, :], sem_out.at[i]).wait()

    def qk(q, r, br, h):
        kt = _slab(u_buf, kv_base(r, 2 * br) + h * (128 // 8) * CT, 256, CT)
        return jnp.dot(q, kt, preferred_element_type=jnp.float32)

    def pv(p, r, br, h):
        vt = _slab(u_buf, kv_base(r, 2 * br + 1) + h * HT, DH, CT)
        return lax.dot_general(vt, p, (((1,), (1,)), ((), ())),
                               preferred_element_type=jnp.float32)

    def qproj(u, br):
        g = _div(u, B)
        if not isinstance(u, int):
            g = jnp.minimum(g, NP - 1)
        x = _slab(u_buf, X_BASE + (2 * _mod(u, B) + br) * XT, SQ, DT)
        q = jnp.dot(x, wq_buf[g, br], preferred_element_type=jnp.float32) * QSCALE
        lane = lax.broadcasted_iota(jnp.int32, (SQ, 256), 1)
        q_sc[_mod(u, 2), br, 0] = jnp.where(lane < DH, q[:, 0:256], 0.0).astype(jnp.bfloat16)
        q_sc[_mod(u, 2), br, 1] = jnp.where(lane >= 64, q[:, 128:384], 0.0).astype(jnp.bfloat16)

    def oproj(o, g, br):
        wo = _slab(u_buf, WO_BASE + (2 * g + br) * WOT, PW, DT)
        return jnp.dot(o, wo, preferred_element_type=jnp.float32)

    for piece in range(16):
        for br in range(2):
            wq_start(0, piece, br)
    x_start(0)
    x_start(1)
    kv_static(-1, 0, NKV)
    acc_sc[...] = jnp.zeros_like(acc_sc)
    kv_static(0, 0, 32)
    wq_wait(0)
    x_wait(0)
    for u in range(2):
        for br in range(2):
            qproj(u, br)
            kv_static(0, 32 + (2 * u + br) * 16, 48 + (2 * u + br) * 16)
    kv_wait(-1, 0)
    s0 = []
    for br in range(2):
        kt = _slab(u_buf, kv_base(-1, 2 * br), DH, CT)
        s0.append(jnp.dot(q_sc[0, br, 0, :, 0:DH], kt, preferred_element_type=jnp.float32))
        for piece in range(8 * br, 8 * br + 8):
            for br2 in range(2):
                wo_start(0, piece, br2)
    for br in range(2):
        p0, l0 = _softmax(s0[br])
        o0_sc[br] = pv(p0, -1, br, 0)
        l0_sc[br] = l0
        for b in range(2 + 3 * br, 5 + 3 * br):
            x_start(b)
    for i in range(W_LEAD - B):
        for k in range(4):
            w_pair_start(1, i, k)
    kv_static(1, 0, MARGIN)
    wo_wait(0)
    x_wait(1)

    def step(r, carry):
        g = _div(r, B)
        b = _mod(r, B)
        gw = _div(r + W_LEAD, B)
        iw = _mod(r + W_LEAD, B)

        def issue(pt):
            for pos in range(MARGIN + pt * PER_PT, MARGIN + (pt + 1) * PER_PT):
                k = pos % NKV
                rr = 1 + pos // NKV
                du = rr + ROUND[k][0]
                if du <= 2:
                    kv_one(r + rr, k)
                else:
                    pl.when(r + du < NU)(lambda: kv_one(r + rr, k))
            if pt % 3 == 1:
                @pl.when(gw < NP)
                def _():
                    w_pair_start(gw, iw, pt // 3)

        @pl.when((b == B - 2) & (g + 1 < NP))
        def _():
            wq_wait(g + 1)
            wo_wait(g + 1)

        kv_wait(r)

        rows = pl.ds(pl.multiple_of(b * SQ, SQ), SQ)
        cur = _mod(r, 2)
        nxt = 1 - cur

        if not (COMPUTE & 1):
            for pt in range(NPT):
                issue(pt)
            return carry

        def accum(o, br):
            y = acc_sc[br, rows, :] + oproj(o, g, br)
            acc_sc[br, rows, :] = y
            if CFG.get('FOLD', 1):
                out_buf[rows, br * D:(br + 1) * D] = y.astype(out_buf.dtype)

        ORDER = CFG['ORDER']
        if ORDER == 0:
            sa1 = qk(q_sc[cur, 0, 1], r, 0, 1)
            issue(0)
            sb1 = qk(q_sc[cur, 1, 1], r, 1, 1)
            issue(1)
            pa1, la1 = _softmax(sa1)
            oa1 = pv(pa1, r, 0, 1)
            issue(2)
            sa0 = qk(q_sc[nxt, 0, 0], r, 0, 0)
            issue(3)
            pb1, lb1 = _softmax(sb1)
            ob1 = pv(pb1, r, 1, 1)
            issue(4)
            qproj(r + 2, 0)
            issue(5)
            sb0 = qk(q_sc[nxt, 1, 0], r, 1, 0)
            issue(6)
            accum(_finish(o0_sc[0], oa1, l0_sc[0], la1), 0)
            issue(7)
            pa0, la0 = _softmax(sa0)
            o0_sc[0] = pv(pa0, r, 0, 0)
            l0_sc[0] = la0
            issue(8)
            qproj(r + 2, 1)
            issue(9)
            accum(_finish(o0_sc[1], ob1, l0_sc[1], lb1), 1)
            issue(10)
            pb0, lb0 = _softmax(sb0)
            o0_sc[1] = pv(pb0, r, 1, 0)
            l0_sc[1] = lb0
            issue(11)
        elif ORDER == 1:
            sa1 = qk(q_sc[cur, 0, 1], r, 0, 1)
            issue(0)
            sb1 = qk(q_sc[cur, 1, 1], r, 1, 1)
            issue(1)
            pa1, la1 = _softmax(sa1)
            oa1 = pv(pa1, r, 0, 1)
            issue(2)
            sa0 = qk(q_sc[nxt, 0, 0], r, 0, 0)
            issue(3)
            pb1, lb1 = _softmax(sb1)
            ob1 = pv(pb1, r, 1, 1)
            issue(4)
            qproj(r + 2, 0)
            issue(5)
            o0a, l0a = o0_sc[0], l0_sc[0]
            pa0, la0 = _softmax(sa0)
            o0_sc[0] = pv(pa0, r, 0, 0)
            l0_sc[0] = la0
            issue(6)
            sb0 = qk(q_sc[nxt, 1, 0], r, 1, 0)
            issue(7)
            accum(_finish(o0a, oa1, l0a, la1), 0)
            issue(8)
            qproj(r + 2, 1)
            issue(9)
            accum(_finish(o0_sc[1], ob1, l0_sc[1], lb1), 1)
            issue(10)
            pb0, lb0 = _softmax(sb0)
            o0_sc[1] = pv(pb0, r, 1, 0)
            l0_sc[1] = lb0
            issue(11)
        elif ORDER == 2:
            sa1 = qk(q_sc[cur, 0, 1], r, 0, 1)
            issue(0)
            qproj(r + 2, 0)
            issue(1)
            pa1, la1 = _softmax(sa1)
            oa1 = pv(pa1, r, 0, 1)
            issue(2)
            sb1 = qk(q_sc[cur, 1, 1], r, 1, 1)
            issue(3)
            qproj(r + 2, 1)
            issue(4)
            pb1, lb1 = _softmax(sb1)
            ob1 = pv(pb1, r, 1, 1)
            issue(5)
            sa0 = qk(q_sc[nxt, 0, 0], r, 0, 0)
            issue(6)
            accum(_finish(o0_sc[0], oa1, l0_sc[0], la1), 0)
            issue(7)
            pa0, la0 = _softmax(sa0)
            o0_sc[0] = pv(pa0, r, 0, 0)
            l0_sc[0] = la0
            issue(8)
            sb0 = qk(q_sc[nxt, 1, 0], r, 1, 0)
            issue(9)
            accum(_finish(o0_sc[1], ob1, l0_sc[1], lb1), 1)
            issue(10)
            pb0, lb0 = _softmax(sb0)
            o0_sc[1] = pv(pb0, r, 1, 0)
            l0_sc[1] = lb0
            issue(11)

        if ORDER == 3:
            sa1 = qk(q_sc[cur, 0, 1], r, 0, 1)
            issue(0)
            sb1 = qk(q_sc[cur, 1, 1], r, 1, 1)
            issue(1)
            pa1, la1 = _softmax(sa1)
            oa1 = pv(pa1, r, 0, 1)
            issue(2)
            sa0 = qk(q_sc[nxt, 0, 0], r, 0, 0)
            issue(3)
            pb1, lb1 = _softmax(sb1)
            ob1 = pv(pb1, r, 1, 1)
            issue(4)
            fa = _finish(o0_sc[0], oa1, l0_sc[0], la1)
            qproj(r + 2, 0)
            issue(5)
            pa0, la0 = _softmax(sa0)
            sb0 = qk(q_sc[nxt, 1, 0], r, 1, 0)
            issue(6)
            o0_sc[0] = pv(pa0, r, 0, 0)
            l0_sc[0] = la0
            issue(7)
            accum(fa, 0)
            issue(8)
            fb = _finish(o0_sc[1], ob1, l0_sc[1], lb1)
            qproj(r + 2, 1)
            issue(9)
            pb0, lb0 = _softmax(sb0)
            accum(fb, 1)
            issue(10)
            o0_sc[1] = pv(pb0, r, 1, 0)
            l0_sc[1] = lb0
            issue(11)
        if ORDER == 4:
            sa1 = qk(q_sc[cur, 0, 1], r, 0, 1)
            issue(0)
            sb1 = qk(q_sc[cur, 1, 1], r, 1, 1)
            issue(1)
            pa1, la1 = _softmax(sa1)
            oa1 = pv(pa1, r, 0, 1)
            issue(2)
            qproj(r + 2, 0)
            issue(3)
            pb1, lb1 = _softmax(sb1)
            ob1 = pv(pb1, r, 1, 1)
            issue(4)
            sa0 = qk(q_sc[nxt, 0, 0], r, 0, 0)
            issue(5)
            accum(_finish(o0_sc[0], oa1, l0_sc[0], la1), 0)
            issue(6)
            pa0, la0 = _softmax(sa0)
            o0_sc[0] = pv(pa0, r, 0, 0)
            l0_sc[0] = la0
            issue(7)
            sb0 = qk(q_sc[nxt, 1, 0], r, 1, 0)
            issue(8)
            qproj(r + 2, 1)
            issue(9)
            accum(_finish(o0_sc[1], ob1, l0_sc[1], lb1), 1)
            issue(10)
            pb0, lb0 = _softmax(sb0)
            o0_sc[1] = pv(pb0, r, 1, 0)
            l0_sc[1] = lb0
            issue(11)
        if ORDER == 5:
            sa1 = qk(q_sc[cur, 0, 1], r, 0, 1)
            issue(0)
            sb1 = qk(q_sc[cur, 1, 1], r, 1, 1)
            issue(1)
            pa1, la1 = _softmax(sa1)
            oa1 = pv(pa1, r, 0, 1)
            issue(2)
            sa0 = qk(q_sc[nxt, 0, 0], r, 0, 0)
            issue(3)
            pb1, lb1 = _softmax(sb1)
            ob1 = pv(pb1, r, 1, 1)
            issue(4)
            sb0 = qk(q_sc[nxt, 1, 0], r, 1, 0)
            issue(5)
            fa = _finish(o0_sc[0], oa1, l0_sc[0], la1)
            pa0, la0 = _softmax(sa0)
            o0_sc[0] = pv(pa0, r, 0, 0)
            l0_sc[0] = la0
            issue(6)
            qproj(r + 2, 0)
            issue(7)
            fb = _finish(o0_sc[1], ob1, l0_sc[1], lb1)
            pb0, lb0 = _softmax(sb0)
            o0_sc[1] = pv(pb0, r, 1, 0)
            l0_sc[1] = lb0
            issue(8)
            qproj(r + 2, 1)
            issue(9)
            accum(fa, 0)
            issue(10)
            accum(fb, 1)
            issue(11)

        if not CFG.get('FOLD', 1):
            @pl.when(g == NP - 1)
            def _():
                out_buf[rows, 0:D] = acc_sc[0, rows, :].astype(out_buf.dtype)
                out_buf[rows, D:2 * D] = acc_sc[1, rows, :].astype(out_buf.dtype)

        return carry

    lax.fori_loop(0, NU - 2, step, 0)

    r = NU - 2
    g = NP - 1
    rows6 = pl.ds((B - 2) * SQ, SQ)
    rows7 = pl.ds((B - 1) * SQ, SQ)
    kv_static(r + 1, MARGIN, NKV)
    TAIL = CFG.get('TAIL', 2)
    if TAIL == 0:
        out_start(0)
    kv_wait(r)
    cur, nxt = r % 2, 1 - r % 2
    sa1 = qk(q_sc[cur, 0, 1], r, 0, 1)
    sb1 = qk(q_sc[cur, 1, 1], r, 1, 1)
    pa1, la1 = _softmax(sa1)
    oa1 = pv(pa1, r, 0, 1)
    sa0 = qk(q_sc[nxt, 0, 0], r, 0, 0)
    if TAIL == 1:
        kv_wait(r + 1, 1)
        out_start(0)
    pb1, lb1 = _softmax(sb1)
    ob1 = pv(pb1, r, 1, 1)
    if TAIL == 2:
        kv_wait(r + 1, 1)
        out_start(0)
    sb0 = qk(q_sc[nxt, 1, 0], r, 1, 0)
    if TAIL == 3:
        kv_wait(r + 1, 1)
        out_start(0)
    oa = _finish(o0_sc[0], oa1, l0_sc[0], la1)
    out_buf[rows6, 0:D] = (acc_sc[0, rows6, :] + oproj(oa, g, 0)).astype(out_buf.dtype)
    if TAIL == 0:
        kv_wait(r + 1, 1)
    sa1 = qk(q_sc[nxt, 0, 1], r + 1, 0, 1)
    pa0, la0 = _softmax(sa0)
    oa0 = pv(pa0, r, 0, 0)
    sb1 = qk(q_sc[nxt, 1, 1], r + 1, 1, 1)
    pb0, lb0 = _softmax(sb0)
    ob0 = pv(pb0, r, 1, 0)
    pa1, la1 = _softmax(sa1)
    oa1 = pv(pa1, r + 1, 0, 1)
    ob = _finish(o0_sc[1], ob1, l0_sc[1], lb1)
    pb1, lb1 = _softmax(sb1)
    ob1 = pv(pb1, r + 1, 1, 1)
    out_buf[rows6, D:2 * D] = (acc_sc[1, rows6, :] + oproj(ob, g, 1)).astype(out_buf.dtype)
    out_start(1)
    oa = _finish(oa0, oa1, la0, la1)
    out_buf[rows7, 0:D] = (acc_sc[0, rows7, :] + oproj(oa, g, 0)).astype(out_buf.dtype)
    ob = _finish(ob0, ob1, lb0, lb1)
    out_buf[rows7, D:2 * D] = (acc_sc[1, rows7, :] + oproj(ob, g, 1)).astype(out_buf.dtype)
    out_start(2)
    for i in range(3):
        out_wait(i)


@jax.jit
def pallas_concat_heads__mha_block_cached__gqa_block_cached__near_ridge_kernel(
    A_x, A_k_cache, A_v_cache, A_wq, A_wo, B_x, B_k_cache, B_v_cache, B_wq, B_wo):
    def tiles(a):
        *lead, rr, cc = a.shape
        a = a.reshape(*lead, rr // 8, 8, cc // 128, 128)
        return jnp.swapaxes(a, -3, -2).reshape(*lead, rr // 8 * (cc // 128), 8, 128)

    def prep(x, k, v, wq, wo):
        return (tiles(x.reshape(B * SQ, D)), wq, tiles(jnp.swapaxes(k, 2, 3)),
                tiles(jnp.swapaxes(v, 2, 3)), tiles(wo))

    any_spec = pl.BlockSpec(memory_space=pl.ANY)
    out = pl.pallas_call(
        _kernel,
        in_specs=[any_spec] * 10,
        out_specs=any_spec,
        out_shape=jax.ShapeDtypeStruct((B * SQ, 2 * D), jnp.bfloat16),
        scratch_shapes=[
            pltpu.VMEM((U_TILES, 8, 128), jnp.bfloat16),
            pltpu.VMEM((NP, 2, D, PW), jnp.bfloat16),
            pltpu.VMEM((2, 2, 2, SQ, 256), jnp.bfloat16),
            pltpu.VMEM((2, DH, SQ), jnp.float32),
            pltpu.VMEM((2, SQ, 1), jnp.float32),
            pltpu.VMEM((2, B * SQ, D), jnp.float32),
            pltpu.VMEM((B * SQ, 2 * D), jnp.bfloat16),
            pltpu.SemaphoreType.DMA((2,)),
            pltpu.SemaphoreType.DMA((2,)),
            pltpu.SemaphoreType.DMA((2,)),
            pltpu.SemaphoreType.DMA((NBUF,)),
            pltpu.SemaphoreType.DMA((3,)),
        ],
        compiler_params=pltpu.CompilerParams(
            vmem_limit_bytes=110 * 1024 * 1024,
            disable_bounds_checks=not CFG.get('CHECKS', 0),
        ),
    )(*prep(A_x, A_k_cache, A_v_cache, A_wq, A_wo), *prep(B_x, B_k_cache, B_v_cache, B_wq, B_wo))
    return out.reshape(B, SQ, 2 * D)
```

```python
import functools
import math

import jax
import jax.numpy as jnp
from jax import lax
import jax.experimental.pallas as pl
import jax.experimental.pallas.tpu as pltpu

B, SQ, D, H, SK, DH = 8, 128, 640, 32, 1024, 192
NP = H // 2
PW = 2 * DH
NU = NP * B
SCALE = (DH ** -0.5) * math.log2(math.e)

NBUF = 4
QLEAD = 4
W_LEAD = 11
OUT_CH = 16
BLK = 16
SHIFT = 13

CT = SK // 128
HT = DH // 8 * CT
DT = D // 128
XT = SQ // 8 * DT
WOT = PW // 8 * DT
QT = H * DH // 128
NRG = D // 8
WQT = NRG * QT


def _cuts(ntiles):
    inner = [SHIFT + BLK * k for k in range(ntiles // BLK) if 0 < SHIFT + BLK * k < ntiles]
    while len(inner) > ntiles // BLK - 1:
        inner = inner[:-1] if SHIFT >= BLK // 2 else inner[1:]
    return [0] + inner + [ntiles]


_KC = _cuts(HT)
_XC = _cuts(XT)
_QC = _cuts(WQT)
NCH = len(_KC) - 1

SLOT_T = 4 * 2 * HT
X_BASE = NBUF * SLOT_T
WO_BASE = X_BASE + B * 2 * XT
U_TILES = WO_BASE + NP * 2 * WOT


def _untile(v):
    n, ct = v.shape[:2]
    return jnp.concatenate([v[:, c].reshape(n * 8, 128) for c in range(ct)], axis=1)


def _slab(u_ref, t0, nrows, ct):
    n = nrows // 8
    return _untile(u_ref[pl.ds(t0, n * ct)].reshape(n, ct, 8, 128))


def _softmax(s):
    m = jnp.max(s, axis=-1, keepdims=True)
    p = jnp.exp2((s - m) * SCALE)
    l = jnp.sum(p, axis=-1, keepdims=True)
    return p.astype(jnp.bfloat16), l


def _finish(ot0, ot1, l0, l1):
    o = jnp.concatenate([ot0, ot1], axis=0).T
    lane = lax.broadcasted_iota(jnp.int32, (SQ, PW), 1)
    inv = jnp.where(lane < DH, 1.0 / l0, 1.0 / l1)
    return (o * inv).astype(jnp.bfloat16)


def _div(v, n):
    return v // n if isinstance(v, int) else lax.shift_right_logical(v, n.bit_length() - 1)


def _mod(v, n):
    return v % n if isinstance(v, int) else v & (n - 1)


def _merge(*lists):
    items = [((i + 0.5) / len(l), n, f) for n, l in enumerate(lists) for i, f in enumerate(l)]
    return [f for _, _, f in sorted(items, key=lambda t: t[:2])]


class _Feeder:
    def __init__(self, plan):
        self.plan = list(plan)

    def __call__(self, n):
        now, self.plan = self.plan[:n], self.plan[n:]
        for f in now:
            f()


def _kernel(xa_hbm, wqa_hbm, ka_hbm, va_hbm, woa_hbm,
            xb_hbm, wqb_hbm, kb_hbm, vb_hbm, wob_hbm,
            out_hbm,
            u_buf, wq_buf, q_sc, o0_sc, l0_sc, acc_sc, out_buf,
            sem_x, sem_wq, sem_wo, sem_kv, sem_out):
    x_hbm = (xa_hbm, xb_hbm)
    wq_hbm = (wqa_hbm, wqb_hbm)
    wo_hbm = (woa_hbm, wob_hbm)
    kv_hbm = (ka_hbm, va_hbm, kb_hbm, vb_hbm)
    part = functools.partial

    def wait_all(ref, sem):
        pltpu.make_async_copy(ref, ref, sem).wait()

    def x_pair(b, c):
        t0, nt = _XC[c], _XC[c + 1] - _XC[c]
        for br in range(2):
            pltpu.make_async_copy(x_hbm[br].at[pl.ds(b * XT + t0, nt)],
                                  u_buf.at[pl.ds(X_BASE + (2 * b + br) * XT + t0, nt)],
                                  sem_x.at[0 if b < QLEAD else 1]).start(priority=br)

    def x_pairs(bs):
        return [part(x_pair, b, c) for b in bs for c in range(len(_XC) - 1)]

    def x_wait(i):
        t0, nt = (0, 2 * QLEAD * XT) if i == 0 else (2 * QLEAD * XT, 2 * (B - QLEAD) * XT)
        wait_all(u_buf.at[pl.ds(X_BASE + t0, nt)], sem_x.at[i])

    def wq_pair(c):
        t0, nt = _QC[c], _QC[c + 1] - _QC[c]
        for br in range(2):
            pltpu.make_async_copy(wq_hbm[br].at[pl.ds(t0, nt)], wq_buf.at[br, pl.ds(t0, nt)],
                                  sem_wq.at[min(c, 1)]).start(priority=br)

    def wq_wait(i):
        t0, nt = (0, _QC[1]) if i == 0 else (_QC[1], WQT - _QC[1])
        wait_all(wq_buf.at[:, pl.ds(t0, nt)], sem_wq.at[i])

    def wo_pair(g, piece):
        nt = WOT // (2 * B)
        for br in range(2):
            pltpu.make_async_copy(wo_hbm[br].at[pl.ds(g * WOT + piece * nt, nt)],
                                  u_buf.at[pl.ds(WO_BASE + (2 * g + br) * WOT + piece * nt, nt)],
                                  sem_wo.at[_mod(g, 2)]).start(priority=br)

    def wo_wait(g):
        wait_all(u_buf.at[pl.ds(WO_BASE + 2 * g * WOT, 2 * WOT)], sem_wo.at[_mod(g, 2)])

    def slot_of(r):
        return _mod(r + 1, NBUF)

    def kv_base(r, h, j):
        return slot_of(r) * SLOT_T + (4 * h + j) * HT

    def kv_pair(r, h, c, br, sem=None):
        u = r + 1 - h
        t0, nt = _KC[c], _KC[c + 1] - _KC[c]
        sem = sem_kv.at[slot_of(r) if sem is None else sem]
        for i in range(2):
            j = 2 * br + i
            pltpu.make_async_copy(kv_hbm[j].at[_mod(u, B), 2 * _div(u, B) + h, pl.ds(t0, nt)],
                                  u_buf.at[pl.ds(kv_base(r, h, j) + t0, nt)],
                                  sem).start(priority=i)

    def kv_round(r):
        return [part(kv_pair, r, h, c, br) for c in range(NCH) for h in (1, 0) for br in range(2)]

    def kv_half(r, h, sem=None):
        return [part(kv_pair, r, h, c, br, sem) for c in range(NCH) for br in range(2)]

    def kv_wait(r):
        wait_all(u_buf.at[pl.ds(kv_base(r, 0, 0), SLOT_T)], sem_kv.at[slot_of(r)])

    def kv_half_wait(r, h, sem=None):
        wait_all(u_buf.at[pl.ds(kv_base(r, h, 0), 4 * HT)],
                 sem_kv.at[slot_of(r) if sem is None else sem])

    out_parts = ((0, (B - 2) * SQ, 6, 0, 2 * D), ((B - 2) * SQ, SQ, 4, 0, 2 * D),
                 ((B - 1) * SQ, SQ, 4, 0, D), ((B - 1) * SQ, SQ, 4, D, D))

    def out_start(i):
        lo, nrows, ns, c0, nc = out_parts[i]
        n = nrows // OUT_CH
        for k in range(n):
            c = (k % ns) * (n // ns) + k // ns
            rows = pl.ds(lo + c * OUT_CH, OUT_CH)
            pltpu.make_async_copy(out_buf.at[rows, pl.ds(c0, nc)], out_hbm.at[rows, pl.ds(c0, nc)],
                                  sem_out.at[i]).start(priority=k % 2)

    def out_wait(i):
        lo, nrows, _, c0, nc = out_parts[i]
        wait_all(out_buf.at[pl.ds(lo, nrows), pl.ds(c0, nc)], sem_out.at[i])

    def qk(r, br, h):
        q = q_sc[_mod(r + 1 - h, QLEAD), br, :, h * 128:h * 128 + 256]
        kt = _slab(u_buf, kv_base(r, h, 2 * br), DH, CT)
        pad = jnp.zeros((256 - DH, SK), kt.dtype)
        kt = jnp.concatenate([kt, pad] if h == 0 else [pad, kt], axis=0)
        return jnp.dot(q, kt, preferred_element_type=jnp.float32)

    def pv(p, r, br, h):
        vt = _slab(u_buf, kv_base(r, h, 2 * br + 1), DH, CT)
        return lax.dot_general(vt, p, (((1,), (1,)), ((), ())),
                               preferred_element_type=jnp.float32)

    def qproj(u, br):
        x = _slab(u_buf, X_BASE + (2 * _mod(u, B) + br) * XT, SQ, DT)
        t0 = _div(u, B) * (PW // 128)
        wq = _untile(jnp.stack(
            [wq_buf[br, pl.ds(t0 + rg * QT, PW // 128)] for rg in range(NRG)]))
        q = jnp.dot(x, wq, preferred_element_type=jnp.float32)
        q_sc[_mod(u, QLEAD), br] = q.astype(jnp.bfloat16)

    def accum(o, u, br):
        row = _mod(u, B) * SQ
        rows = pl.ds(row if isinstance(row, int) else pl.multiple_of(row, SQ), SQ)
        wo = _slab(u_buf, WO_BASE + (2 * _div(u, B) + br) * WOT, PW, DT)
        y = acc_sc[br, rows, :] + jnp.dot(o, wo, preferred_element_type=jnp.float32)
        if not (isinstance(u, int) and u >= NU - B):
            acc_sc[br, rows, :] = y
        out_buf[rows, br * D:(br + 1) * D] = y.astype(out_buf.dtype)

    def body(r, issue, with_q):
        sa1 = qk(r, 0, 1)
        issue(0)
        sb1 = qk(r, 1, 1)
        issue(1)
        pa1, la1 = _softmax(sa1)
        oa1 = pv(pa1, r, 0, 1)
        issue(2)
        sa0 = qk(r, 0, 0)
        issue(3)
        pb1, lb1 = _softmax(sb1)
        ob1 = pv(pb1, r, 1, 1)
        issue(4)
        fa = _finish(o0_sc[0], oa1, l0_sc[0], la1)
        if with_q:
            qproj(r + QLEAD, 0)
        issue(5)
        pa0, la0 = _softmax(sa0)
        sb0 = qk(r, 1, 0)
        issue(6)
        o0_sc[0] = pv(pa0, r, 0, 0)
        l0_sc[0] = la0
        issue(7)
        accum(fa, r, 0)
        issue(8)
        fb = _finish(o0_sc[1], ob1, l0_sc[1], lb1)
        if with_q:
            qproj(r + QLEAD, 1)
        issue(9)
        pb0, lb0 = _softmax(sb0)
        accum(fb, r, 1)
        issue(10)
        o0_sc[1] = pv(pb0, r, 1, 0)
        l0_sc[1] = lb0
        issue(11)

    nq, nsub = len(_QC) - 1, 4
    for i in range(nq // nsub):
        for sub in range(nsub):
            wq_pair(sub * (nq // nsub) + i)
    acc_sc[...] = jnp.zeros_like(acc_sc)
    wq_wait(0)

    first = _merge(x_pairs(range(QLEAD)), kv_half(-1, 0))
    feed = _Feeder(
        first
        + _merge(kv_round(0), [part(wo_pair, 0, p) for p in range(2 * B)],
                 x_pairs(range(QLEAD, B)))
        + _merge(kv_round(1), [part(wo_pair, 1, p) for p in range(2 * (W_LEAD - B))]))
    feed(len(first) + 40)
    wq_wait(1)
    x_wait(0)
    kv_half_wait(-1, 0)
    for u in range(2):
        for br in range(2):
            qproj(u, br)
            feed(5)
    s0 = []
    for br in range(2):
        s0.append(qk(-1, br, 0))
        feed(5)
    for br in range(2):
        for u in range(2, QLEAD):
            qproj(u, br)
            feed(5)
        p0, l0 = _softmax(s0[br])
        o0_sc[br] = pv(p0, -1, br, 0)
        l0_sc[br] = l0
        feed(5)
    feed(len(feed.plan))
    wo_wait(0)
    x_wait(1)

    def step(r, carry):
        gw = _div(r + W_LEAD, B)
        iw = _mod(r + W_LEAD, B)
        plan = kv_round(r + 2)

        def issue(pt):
            for f in plan[4 * pt:4 * pt + 4]:
                f()
            if pt in (3, 9):
                pl.when(gw < NP)(part(wo_pair, gw, 2 * iw + pt // 6))

        pl.when(_mod(r, B) == B - 1)(part(wo_wait, _div(r, B) + 1))
        kv_wait(r)
        body(r, issue, True)
        return carry

    lax.fori_loop(0, NU - QLEAD, step, 0)

    r, r2, r3 = NU - 3, NU - 2, NU - 1
    feed = _Feeder(kv_half(r2, 1) + kv_half(r2, 0, NBUF) + kv_half(r3, 1))
    kv_wait(r - 1)
    body(r - 1, lambda pt: feed(4), False)

    kv_wait(r)
    sa1 = qk(r, 0, 1)
    feed(4)
    sb1 = qk(r, 1, 1)
    feed(4)
    pa1, la1 = _softmax(sa1)
    oa1 = pv(pa1, r, 0, 1)
    feed(4)
    sa0 = qk(r, 0, 0)
    feed(4)
    pb1, lb1 = _softmax(sb1)
    ob1 = pv(pb1, r, 1, 1)
    feed(4)
    fa = _finish(o0_sc[0], oa1, l0_sc[0], la1)
    pa0, la0 = _softmax(sa0)
    sb0 = qk(r, 1, 0)
    feed(len(feed.plan))
    oa0 = pv(pa0, r, 0, 0)
    fb = _finish(o0_sc[1], ob1, l0_sc[1], lb1)
    pb0, lb0 = _softmax(sb0)
    accum(fa, r, 0)

    kv_half_wait(r2, 1)
    sc1 = qk(r2, 0, 1)
    ob0 = pv(pb0, r, 1, 0)
    sd1 = qk(r2, 1, 1)
    pc1, lc1 = _softmax(sc1)
    accum(fb, r, 1)
    oc1 = pv(pc1, r2, 0, 1)
    pd1, ld1 = _softmax(sd1)

    kv_half_wait(r2, 0, NBUF)
    out_start(0)
    sc0 = qk(r2, 0, 0)
    fc = _finish(oa0, oc1, la0, lc1)
    od1 = pv(pd1, r2, 1, 1)
    sd0 = qk(r2, 1, 0)
    pc0, lc0 = _softmax(sc0)
    accum(fc, r2, 0)
    oc0 = pv(pc0, r2, 0, 0)
    fd = _finish(ob0, od1, lb0, ld1)
    pd0, ld0 = _softmax(sd0)

    kv_half_wait(r3, 1)
    se1 = qk(r3, 0, 1)
    od0 = pv(pd0, r2, 1, 0)
    sf1 = qk(r3, 1, 1)
    pe1, le1 = _softmax(se1)
    oe1 = pv(pe1, r3, 0, 1)
    accum(fd, r2, 1)
    out_start(1)
    pf1, lf1 = _softmax(sf1)
    of1 = pv(pf1, r3, 1, 1)
    accum(_finish(oc0, oe1, lc0, le1), r3, 0)
    out_start(2)
    accum(_finish(od0, of1, ld0, lf1), r3, 1)
    out_start(3)
    for i in range(len(out_parts)):
        out_wait(i)


@jax.jit
def pallas_concat_heads__mha_block_cached__gqa_block_cached__near_ridge_kernel(
    A_x: jax.Array,
    A_k_cache: jax.Array,
    A_v_cache: jax.Array,
    A_wq: jax.Array,
    A_wo: jax.Array,
    B_x: jax.Array,
    B_k_cache: jax.Array,
    B_v_cache: jax.Array,
    B_wq: jax.Array,
    B_wo: jax.Array,
):
    for kv in (A_k_cache, A_v_cache, B_k_cache, B_v_cache):
        assert kv.shape == (B, H, SK, DH)

    def tiles(a):
        *lead, rr, cc = a.shape
        a = a.reshape(*lead, rr // 8, 8, cc // 128, 128)
        return jnp.swapaxes(a, -3, -2).reshape(*lead, rr // 8 * (cc // 128), 8, 128)

    def prep(x, k, v, wq, wo):
        return (tiles(x.reshape(B * SQ, D)), tiles(wq), tiles(jnp.swapaxes(k, 2, 3)),
                tiles(jnp.swapaxes(v, 2, 3)), tiles(wo))

    any_spec = pl.BlockSpec(memory_space=pl.ANY)
    out = pl.pallas_call(
        _kernel,
        in_specs=[any_spec] * 10,
        out_specs=any_spec,
        out_shape=jax.ShapeDtypeStruct((B * SQ, 2 * D), jnp.bfloat16),
        scratch_shapes=[
            pltpu.VMEM((U_TILES, 8, 128), jnp.bfloat16),
            pltpu.VMEM((2, WQT, 8, 128), jnp.bfloat16),
            pltpu.VMEM((QLEAD, 2, SQ, PW), jnp.bfloat16),
            pltpu.VMEM((2, DH, SQ), jnp.float32),
            pltpu.VMEM((2, SQ, 1), jnp.float32),
            pltpu.VMEM((2, B * SQ, D), jnp.float32),
            pltpu.VMEM((B * SQ, 2 * D), jnp.bfloat16),
            pltpu.SemaphoreType.DMA((2,)),
            pltpu.SemaphoreType.DMA((2,)),
            pltpu.SemaphoreType.DMA((2,)),
            pltpu.SemaphoreType.DMA((NBUF + 1,)),
            pltpu.SemaphoreType.DMA((4,)),
        ],
        compiler_params=pltpu.CompilerParams(
            vmem_limit_bytes=100 * 1024 * 1024,
            disable_bounds_checks=True,
        ),
    )(*prep(A_x, A_k_cache, A_v_cache, A_wq, A_wo), *prep(B_x, B_k_cache, B_v_cache, B_wq, B_wo))
    return out.reshape(B, SQ, 2 * D)
```

```python
import functools
import math

import jax
import jax.numpy as jnp
from jax import lax
import jax.experimental.pallas as pl
import jax.experimental.pallas.tpu as pltpu

B, SQ, D, H, SK, DH = 8, 128, 640, 32, 1024, 192
NP = H // 2
PW = 2 * DH
NU = NP * B
SCALE = (DH ** -0.5) * math.log2(math.e)

NBUF = 4
QLEAD = 4
W_LEAD = 11
OUT_CH = 16
BLK = 16
SHIFT = 13

CT = SK // 128
HT = DH // 8 * CT
DT = D // 128
XT = SQ // 8 * DT
WOT = PW // 8 * DT
QT = H * DH // 128
NRG = D // 8
WQT = NRG * QT


def _cuts(ntiles):
    inner = [SHIFT + BLK * k for k in range(ntiles // BLK) if 0 < SHIFT + BLK * k < ntiles]
    while len(inner) > ntiles // BLK - 1:
        inner = inner[:-1] if SHIFT >= BLK // 2 else inner[1:]
    return [0] + inner + [ntiles]


_KC = _cuts(HT)
_XC = _cuts(XT)
_QC = _cuts(WQT)
NCH = len(_KC) - 1

SLOT_T = 4 * 2 * HT
X_BASE = NBUF * SLOT_T
WO_BASE = X_BASE + B * 2 * XT
U_TILES = WO_BASE + NP * 2 * WOT


def _untile(v):
    n, ct = v.shape[:2]
    return jnp.concatenate([v[:, c].reshape(n * 8, 128) for c in range(ct)], axis=1)


def _slab(u_ref, t0, nrows, ct):
    n = nrows // 8
    return _untile(u_ref[pl.ds(t0, n * ct)].reshape(n, ct, 8, 128))


def _softmax(s):
    m = jnp.max(s, axis=-1, keepdims=True)
    p = jnp.exp2((s - m) * SCALE)
    l = jnp.sum(p, axis=-1, keepdims=True)
    return p.astype(jnp.bfloat16), l


def _finish(ot0, ot1, l0, l1):
    o = jnp.concatenate([ot0, ot1], axis=0).T
    lane = lax.broadcasted_iota(jnp.int32, (SQ, PW), 1)
    inv = jnp.where(lane < DH, 1.0 / l0, 1.0 / l1)
    return (o * inv).astype(jnp.bfloat16)


def _div(v, n):
    return v // n if isinstance(v, int) else lax.shift_right_logical(v, n.bit_length() - 1)


def _mod(v, n):
    return v % n if isinstance(v, int) else v & (n - 1)


def _merge(*lists):
    items = [((i + 0.5) / len(l), n, f) for n, l in enumerate(lists) for i, f in enumerate(l)]
    return [f for _, _, f in sorted(items, key=lambda t: t[:2])]


class _Feeder:
    def __init__(self, plan):
        self.plan = list(plan)

    def __call__(self, n):
        now, self.plan = self.plan[:n], self.plan[n:]
        for f in now:
            f()


def _kernel(xa_hbm, wqa_hbm, ka_hbm, va_hbm, woa_hbm,
            xb_hbm, wqb_hbm, kb_hbm, vb_hbm, wob_hbm,
            out_hbm,
            u_buf, wq_buf, q_sc, o0_sc, l0_sc, acc_sc, out_buf,
            sem_x, sem_wq, sem_wo, sem_kv, sem_out):
    x_hbm = (xa_hbm, xb_hbm)
    wq_hbm = (wqa_hbm, wqb_hbm)
    wo_hbm = (woa_hbm, wob_hbm)
    kv_hbm = (ka_hbm, va_hbm, kb_hbm, vb_hbm)
    part = functools.partial

    def wait_all(ref, sem):
        pltpu.make_async_copy(ref, ref, sem).wait()

    def x_pair(b, c):
        t0, nt = _XC[c], _XC[c + 1] - _XC[c]
        for br in range(2):
            pltpu.make_async_copy(x_hbm[br].at[pl.ds(b * XT + t0, nt)],
                                  u_buf.at[pl.ds(X_BASE + (2 * b + br) * XT + t0, nt)],
                                  sem_x.at[0 if b < QLEAD else 1]).start(priority=br)

    def x_pairs(bs):
        return [part(x_pair, b, c) for b in bs for c in range(len(_XC) - 1)]

    def x_wait(i):
        t0, nt = (0, 2 * QLEAD * XT) if i == 0 else (2 * QLEAD * XT, 2 * (B - QLEAD) * XT)
        wait_all(u_buf.at[pl.ds(X_BASE + t0, nt)], sem_x.at[i])

    def wq_pair(c):
        t0, nt = _QC[c], _QC[c + 1] - _QC[c]
        for br in range(2):
            pltpu.make_async_copy(wq_hbm[br].at[pl.ds(t0, nt)], wq_buf.at[br, pl.ds(t0, nt)],
                                  sem_wq.at[min(c, 1)]).start(priority=br)

    def wq_wait(i):
        t0, nt = (0, _QC[1]) if i == 0 else (_QC[1], WQT - _QC[1])
        wait_all(wq_buf.at[:, pl.ds(t0, nt)], sem_wq.at[i])

    def wo_pair(g, piece):
        nt = WOT // (2 * B)
        for br in range(2):
            pltpu.make_async_copy(wo_hbm[br].at[pl.ds(g * WOT + piece * nt, nt)],
                                  u_buf.at[pl.ds(WO_BASE + (2 * g + br) * WOT + piece * nt, nt)],
                                  sem_wo.at[_mod(g, 2)]).start(priority=br)

    def wo_wait(g):
        wait_all(u_buf.at[pl.ds(WO_BASE + 2 * g * WOT, 2 * WOT)], sem_wo.at[_mod(g, 2)])

    def slot_of(r):
        return _mod(r + 1, NBUF)

    def kv_base(r, h, j):
        return slot_of(r) * SLOT_T + (4 * h + j) * HT

    def kv_pair(r, h, c, br, sem=None):
        u = r + 1 - h
        t0, nt = _KC[c], _KC[c + 1] - _KC[c]
        sem = sem_kv.at[slot_of(r) if sem is None else sem]
        for i in range(2):
            j = 2 * br + i
            pltpu.make_async_copy(kv_hbm[j].at[_mod(u, B), 2 * _div(u, B) + h, pl.ds(t0, nt)],
                                  u_buf.at[pl.ds(kv_base(r, h, j) + t0, nt)],
                                  sem).start(priority=i)

    def kv_round(r):
        return [part(kv_pair, r, h, c, br) for c in range(NCH) for h in (1, 0) for br in range(2)]

    def kv_half(r, h, sem=None):
        return [part(kv_pair, r, h, c, br, sem) for c in range(NCH) for br in range(2)]

    def kv_wait(r):
        wait_all(u_buf.at[pl.ds(kv_base(r, 0, 0), SLOT_T)], sem_kv.at[slot_of(r)])

    def kv_half_wait(r, h, sem=None):
        wait_all(u_buf.at[pl.ds(kv_base(r, h, 0), 4 * HT)],
                 sem_kv.at[slot_of(r) if sem is None else sem])

    out_parts = ((0, (B - 2) * SQ, 6, 0, 2 * D), ((B - 2) * SQ, SQ, 4, 0, 2 * D),
                 ((B - 1) * SQ, SQ, 4, 0, D), ((B - 1) * SQ, SQ, 4, D, D))

    def out_start(i):
        lo, nrows, ns, c0, nc = out_parts[i]
        n = nrows // OUT_CH
        for k in range(n):
            c = (k % ns) * (n // ns) + k // ns
            rows = pl.ds(lo + c * OUT_CH, OUT_CH)
            pltpu.make_async_copy(out_buf.at[rows, pl.ds(c0, nc)], out_hbm.at[rows, pl.ds(c0, nc)],
                                  sem_out.at[i]).start(priority=k % 2)

    def out_wait(i):
        lo, nrows, _, c0, nc = out_parts[i]
        wait_all(out_buf.at[pl.ds(lo, nrows), pl.ds(c0, nc)], sem_out.at[i])

    def qk(r, br, h):
        q = q_sc[_mod(r + 1 - h, QLEAD), br, :, h * 128:h * 128 + 256]
        kt = _slab(u_buf, kv_base(r, h, 2 * br), DH, CT)
        pad = jnp.zeros((256 - DH, SK), kt.dtype)
        kt = jnp.concatenate([kt, pad] if h == 0 else [pad, kt], axis=0)
        return jnp.dot(q, kt, preferred_element_type=jnp.float32)

    def pv(p, r, br, h):
        vt = _slab(u_buf, kv_base(r, h, 2 * br + 1), DH, CT)
        return lax.dot_general(vt, p, (((1,), (1,)), ((), ())),
                               preferred_element_type=jnp.float32)

    def qproj(u, br):
        x = _slab(u_buf, X_BASE + (2 * _mod(u, B) + br) * XT, SQ, DT)
        t0 = _div(u, B) * (PW // 128)
        wq = _untile(jnp.stack(
            [wq_buf[br, pl.ds(t0 + rg * QT, PW // 128)] for rg in range(NRG)]))
        q = jnp.dot(x, wq, preferred_element_type=jnp.float32)
        q_sc[_mod(u, QLEAD), br] = q.astype(jnp.bfloat16)

    def accum(o, u, br):
        row = _mod(u, B) * SQ
        rows = pl.ds(row if isinstance(row, int) else pl.multiple_of(row, SQ), SQ)
        wo = _slab(u_buf, WO_BASE + (2 * _div(u, B) + br) * WOT, PW, DT)
        y = acc_sc[br, rows, :] + jnp.dot(o, wo, preferred_element_type=jnp.float32)
        if not (isinstance(u, int) and u >= NU - B):
            acc_sc[br, rows, :] = y
        out_buf[rows, br * D:(br + 1) * D] = y.astype(out_buf.dtype)

    def body(r, issue):
        sa1 = qk(r, 0, 1)
        issue(0)
        sb1 = qk(r, 1, 1)
        issue(1)
        pa1, la1 = _softmax(sa1)
        sa0 = qk(r, 0, 0)
        issue(2)
        pb1, lb1 = _softmax(sb1)
        oa1 = pv(pa1, r, 0, 1)
        issue(3)
        ob1 = pv(pb1, r, 1, 1)
        issue(4)
        fa = _finish(o0_sc[0], oa1, l0_sc[0], la1)
        qproj(r + QLEAD, 0)
        issue(5)
        pa0, la0 = _softmax(sa0)
        accum(fa, r, 0)
        issue(6)
        sb0 = qk(r, 1, 0)
        issue(7)
        fb = _finish(o0_sc[1], ob1, l0_sc[1], lb1)
        o0_sc[0] = pv(pa0, r, 0, 0)
        l0_sc[0] = la0
        issue(8)
        qproj(r + QLEAD, 1)
        issue(9)
        pb0, lb0 = _softmax(sb0)
        accum(fb, r, 1)
        issue(10)
        o0_sc[1] = pv(pb0, r, 1, 0)
        l0_sc[1] = lb0
        issue(11)

    nq, nsub = len(_QC) - 1, 4
    for i in range(nq // nsub):
        for sub in range(nsub):
            wq_pair(sub * (nq // nsub) + i)
    acc_sc[...] = jnp.zeros_like(acc_sc)
    wq_wait(0)

    first = _merge(x_pairs(range(QLEAD)), kv_half(-1, 0))
    feed = _Feeder(
        first
        + _merge(kv_round(0), [part(wo_pair, 0, p) for p in range(2 * B)],
                 x_pairs(range(QLEAD, B)))
        + _merge(kv_round(1), [part(wo_pair, 1, p) for p in range(2 * (W_LEAD - B))]))
    feed(len(first) + 60)
    wq_wait(1)
    x_wait(0)
    kv_half_wait(-1, 0)
    for u in range(2):
        for br in range(2):
            qproj(u, br)
            feed(4)
    s0 = []
    for br in range(2):
        s0.append(qk(-1, br, 0))
        feed(4)
    for br in range(2):
        for u in range(2, QLEAD):
            qproj(u, br)
            feed(4)
        p0, l0 = _softmax(s0[br])
        o0_sc[br] = pv(p0, -1, br, 0)
        l0_sc[br] = l0
        feed(4)
    feed(len(feed.plan))
    wo_wait(0)
    x_wait(1)

    def step(r, carry):
        gw = _div(r + W_LEAD, B)
        iw = _mod(r + W_LEAD, B)
        plan = kv_round(r + 2)

        def issue(pt):
            for f in plan[4 * pt:4 * pt + 4]:
                f()
            if pt in (3, 9):
                pl.when(gw < NP)(part(wo_pair, gw, 2 * iw + pt // 6))

        pl.when(_mod(r, B) == B - 1)(part(wo_wait, _div(r, B) + 1))
        kv_wait(r)
        body(r, issue)
        return carry

    r0 = NU - QLEAD
    lax.fori_loop(0, r0 - 1, step, 0)

    halves = [(r, h) for r in range(r0 + 1, NU) for h in (1, 0)][:-1]
    half_sem = {(r, h): (None if h == 1 else NBUF + r - r0 - 1) for r, h in halves}
    feed = _Feeder([f for r, h in halves for f in kv_half(r, h, half_sem[r, h])])
    kv_wait(r0 - 1)
    body(r0 - 1, lambda pt: feed(4))

    kv_wait(r0)
    sa1 = qk(r0, 0, 1)
    feed(4)
    sb1 = qk(r0, 1, 1)
    feed(4)
    pa1, la1 = _softmax(sa1)
    oa1 = pv(pa1, r0, 0, 1)
    feed(4)
    sa0 = qk(r0, 0, 0)
    feed(4)
    pb1, lb1 = _softmax(sb1)
    ob1 = pv(pb1, r0, 1, 1)
    feed(4)
    fa = _finish(o0_sc[0], oa1, l0_sc[0], la1)
    pa0, la0 = _softmax(sa0)
    sb0 = qk(r0, 1, 0)
    feed(4)
    done = {(r0 + 1, 0, 0): (pv(pa0, r0, 0, 0), la0)}
    feed(4)
    ready = [(_finish(o0_sc[1], ob1, l0_sc[1], lb1), r0, 1)]
    prev = _softmax(sb0) + (r0, 0)
    accum(fa, r0, 0)
    feed(4)

    def complete(u, br):
        (o0, l0), (o1, l1) = done[u, br, 0], done[u, br, 1]
        ready.append((_finish(o0, o1, l0, l1), u, br))

    def project():
        o, u, br = ready.pop(0)
        accum(o, u, br)
        if (u, br) == (NU - 2, 1):
            out_start(1)
        elif u == NU - 1:
            out_start(2 + br)

    def prev_pv(p, l, r, h):
        done[r + 1 - h, 1, h] = (pv(p, r, 1, h), l)
        if h == 1:
            complete(r, 1)

    for r, h in halves:
        last = (r, h) == halves[-1]
        if not last:
            kv_half_wait(r, h, half_sem[r, h])
        sx = qk(r, 0, h)
        feed(4)
        if h == 0:
            complete(r, 0)
        prev_pv(*prev)
        feed(4)
        if (r, h) == halves[-2]:
            assert not feed.plan and all(u >= NU - 2 for _, u, _ in ready)
            kv_half_wait(*halves[-1])
            out_start(0)
        sy = qk(r, 1, h)
        feed(4)
        px, lx = _softmax(sx)
        if not last:
            project()
            feed(4)
        done[r + 1 - h, 0, h] = (pv(px, r, 0, h), lx)
        feed(4)
        if last:
            project()
            complete(r, 0)
        prev = _softmax(sy) + (r, h)
    prev_pv(*prev)
    while ready:
        project()
    for i in range(len(out_parts)):
        out_wait(i)


@jax.jit
def pallas_concat_heads__mha_block_cached__gqa_block_cached__near_ridge_kernel(
    A_x: jax.Array,
    A_k_cache: jax.Array,
    A_v_cache: jax.Array,
    A_wq: jax.Array,
    A_wo: jax.Array,
    B_x: jax.Array,
    B_k_cache: jax.Array,
    B_v_cache: jax.Array,
    B_wq: jax.Array,
    B_wo: jax.Array,
):
    for kv in (A_k_cache, A_v_cache, B_k_cache, B_v_cache):
        assert kv.shape == (B, H, SK, DH)

    def tiles(a):
        *lead, rr, cc = a.shape
        a = a.reshape(*lead, rr // 8, 8, cc // 128, 128)
        return jnp.swapaxes(a, -3, -2).reshape(*lead, rr // 8 * (cc // 128), 8, 128)

    def prep(x, k, v, wq, wo):
        return (tiles(x.reshape(B * SQ, D)), tiles(wq), tiles(jnp.swapaxes(k, 2, 3)),
                tiles(jnp.swapaxes(v, 2, 3)), tiles(wo))

    any_spec = pl.BlockSpec(memory_space=pl.ANY)
    out = pl.pallas_call(
        _kernel,
        in_specs=[any_spec] * 10,
        out_specs=any_spec,
        out_shape=jax.ShapeDtypeStruct((B * SQ, 2 * D), jnp.bfloat16),
        scratch_shapes=[
            pltpu.VMEM((U_TILES, 8, 128), jnp.bfloat16),
            pltpu.VMEM((2, WQT, 8, 128), jnp.bfloat16),
            pltpu.VMEM((QLEAD, 2, SQ, PW), jnp.bfloat16),
            pltpu.VMEM((2, DH, SQ), jnp.float32),
            pltpu.VMEM((2, SQ, 1), jnp.float32),
            pltpu.VMEM((2, B * SQ, D), jnp.float32),
            pltpu.VMEM((B * SQ, 2 * D), jnp.bfloat16),
            pltpu.SemaphoreType.DMA((2,)),
            pltpu.SemaphoreType.DMA((2,)),
            pltpu.SemaphoreType.DMA((2,)),
            pltpu.SemaphoreType.DMA((NBUF + QLEAD - 2,)),
            pltpu.SemaphoreType.DMA((4,)),
        ],
        compiler_params=pltpu.CompilerParams(
            vmem_limit_bytes=100 * 1024 * 1024,
            disable_bounds_checks=True,
        ),
    )(*prep(A_x, A_k_cache, A_v_cache, A_wq, A_wo), *prep(B_x, B_k_cache, B_v_cache, B_wq, B_wo))
    return out.reshape(B, SQ, 2 * D)
```

```python
import functools
import math

import jax
import jax.numpy as jnp
from jax import lax
import jax.experimental.pallas as pl
import jax.experimental.pallas.tpu as pltpu

B, SQ, D, H, SK, DH = 8, 128, 640, 32, 1024, 192
NP = H // 2
PW = 2 * DH
NU = NP * B
SCALE = (DH ** -0.5) * math.log2(math.e)

NBUF = 4
QLEAD = 5
QRING = 8
W_LEAD = 11
OUT_CH = 16
BLK = 16
SHIFT = 13

CT = SK // 128
HT = DH // 8 * CT
DT = D // 128
XT = SQ // 8 * DT
WOT = PW // 8 * DT
QT = H * DH // 128
NRG = D // 8
WQT = NRG * QT


def _cuts(ntiles):
    inner = [SHIFT + BLK * k for k in range(ntiles // BLK) if 0 < SHIFT + BLK * k < ntiles]
    while len(inner) > ntiles // BLK - 1:
        inner = inner[:-1] if SHIFT >= BLK // 2 else inner[1:]
    return [0] + inner + [ntiles]


_KC = _cuts(HT)
_XC = _cuts(XT)
_QC = _cuts(WQT)
NCH = len(_KC) - 1

SLOT_T = 4 * 2 * HT
X_BASE = NBUF * SLOT_T
WO_BASE = X_BASE + B * 2 * XT
U_TILES = WO_BASE + NP * 2 * WOT


def _untile(v):
    n, ct = v.shape[:2]
    return jnp.concatenate([v[:, c].reshape(n * 8, 128) for c in range(ct)], axis=1)


def _slab(u_ref, t0, nrows, ct):
    n = nrows // 8
    return _untile(u_ref[pl.ds(t0, n * ct)].reshape(n, ct, 8, 128))


def _softmax(s):
    m = jnp.max(s, axis=-1, keepdims=True)
    p = jnp.exp2((s - m) * SCALE)
    l = jnp.sum(p, axis=-1, keepdims=True)
    return p.astype(jnp.bfloat16), l


def _finish(ot0, ot1, l0, l1):
    o = jnp.concatenate([ot0, ot1], axis=0).T
    lane = lax.broadcasted_iota(jnp.int32, (SQ, PW), 1)
    inv = jnp.where(lane < DH, 1.0 / l0, 1.0 / l1)
    return (o * inv).astype(jnp.bfloat16)


def _div(v, n):
    return v // n if isinstance(v, int) else lax.shift_right_logical(v, n.bit_length() - 1)


def _mod(v, n):
    return v % n if isinstance(v, int) else v & (n - 1)


def _merge(*lists):
    items = [((i + 0.5) / len(l), n, f) for n, l in enumerate(lists) for i, f in enumerate(l)]
    return [f for _, _, f in sorted(items, key=lambda t: t[:2])]


class _Feeder:
    def __init__(self, plan):
        self.plan = list(plan)

    def __call__(self, n):
        now, self.plan = self.plan[:n], self.plan[n:]
        for f in now:
            f()


def _kernel(xa_hbm, wqa_hbm, ka_hbm, va_hbm, woa_hbm,
            xb_hbm, wqb_hbm, kb_hbm, vb_hbm, wob_hbm,
            out_hbm,
            u_buf, wq_buf, q_sc, o0_sc, l0_sc, acc_sc, out_buf,
            sem_x, sem_wq, sem_wo, sem_kv, sem_out):
    x_hbm = (xa_hbm, xb_hbm)
    wq_hbm = (wqa_hbm, wqb_hbm)
    wo_hbm = (woa_hbm, wob_hbm)
    kv_hbm = (ka_hbm, va_hbm, kb_hbm, vb_hbm)
    part = functools.partial

    def wait_all(ref, sem):
        pltpu.make_async_copy(ref, ref, sem).wait()

    def x_pair(b, c):
        t0, nt = _XC[c], _XC[c + 1] - _XC[c]
        for br in range(2):
            pltpu.make_async_copy(x_hbm[br].at[pl.ds(b * XT + t0, nt)],
                                  u_buf.at[pl.ds(X_BASE + (2 * b + br) * XT + t0, nt)],
                                  sem_x.at[0 if b < QLEAD else 1]).start(priority=br)

    def x_pairs(bs):
        return [part(x_pair, b, c) for b in bs for c in range(len(_XC) - 1)]

    def x_wait(i):
        t0, nt = (0, 2 * QLEAD * XT) if i == 0 else (2 * QLEAD * XT, 2 * (B - QLEAD) * XT)
        wait_all(u_buf.at[pl.ds(X_BASE + t0, nt)], sem_x.at[i])

    def wq_pair(c):
        t0, nt = _QC[c], _QC[c + 1] - _QC[c]
        for br in range(2):
            pltpu.make_async_copy(wq_hbm[br].at[pl.ds(t0, nt)], wq_buf.at[br, pl.ds(t0, nt)],
                                  sem_wq.at[min(c, 1)]).start(priority=br)

    def wq_wait(i):
        t0, nt = (0, _QC[1]) if i == 0 else (_QC[1], WQT - _QC[1])
        wait_all(wq_buf.at[:, pl.ds(t0, nt)], sem_wq.at[i])

    def wo_pair(g, piece):
        nt = WOT // (2 * B)
        for br in range(2):
            pltpu.make_async_copy(wo_hbm[br].at[pl.ds(g * WOT + piece * nt, nt)],
                                  u_buf.at[pl.ds(WO_BASE + (2 * g + br) * WOT + piece * nt, nt)],
                                  sem_wo.at[_mod(g, 2)]).start(priority=br)

    def wo_wait(g):
        wait_all(u_buf.at[pl.ds(WO_BASE + 2 * g * WOT, 2 * WOT)], sem_wo.at[_mod(g, 2)])

    def slot_of(r):
        return _mod(r + 1, NBUF)

    def kv_base(r, h, kv, br):
        return slot_of(r) * SLOT_T + (4 * h + 2 * kv + br) * HT

    def kv_pair(r, h, c, kv, sem=None):
        u = r + 1 - h
        t0, nt = _KC[c], _KC[c + 1] - _KC[c]
        sem = sem_kv.at[slot_of(r) if sem is None else sem]
        for br in range(2):
            pltpu.make_async_copy(
                kv_hbm[2 * br + kv].at[_mod(u, B), 2 * _div(u, B) + h, pl.ds(t0, nt)],
                u_buf.at[pl.ds(kv_base(r, h, kv, br) + t0, nt)], sem).start(priority=br)

    def kv_round(r):
        return [part(kv_pair, r, h, c, kv) for c in range(NCH) for h in (1, 0) for kv in range(2)]

    def kv_half(r, h, sem=None, kvs=(0, 1)):
        return [part(kv_pair, r, h, c, kv, sem) for c in range(NCH) for kv in kvs]

    def kv_wait(r):
        wait_all(u_buf.at[pl.ds(kv_base(r, 0, 0, 0), SLOT_T)], sem_kv.at[slot_of(r)])

    def kv_half_wait(r, h, sem=None, kvs=(0, 1)):
        wait_all(u_buf.at[pl.ds(kv_base(r, h, kvs[0], 0), 2 * len(kvs) * HT)],
                 sem_kv.at[slot_of(r) if sem is None else sem])

    out_parts = ((0, (B - 1) * SQ, 7, 0, 2 * D),
                 ((B - 1) * SQ, SQ, 4, 0, D), ((B - 1) * SQ, SQ, 4, D, D))

    def out_start(i):
        lo, nrows, ns, c0, nc = out_parts[i]
        n = nrows // OUT_CH
        for k in range(n):
            c = (k % ns) * (n // ns) + k // ns
            rows = pl.ds(lo + c * OUT_CH, OUT_CH)
            pltpu.make_async_copy(out_buf.at[rows, pl.ds(c0, nc)], out_hbm.at[rows, pl.ds(c0, nc)],
                                  sem_out.at[i]).start(priority=k % 2)

    def out_wait(i):
        lo, nrows, _, c0, nc = out_parts[i]
        wait_all(out_buf.at[pl.ds(lo, nrows), pl.ds(c0, nc)], sem_out.at[i])

    def qk(r, br, h):
        q = q_sc[_mod(r + 1 - h, QRING), br, :, h * 128:h * 128 + 256]
        kt = _slab(u_buf, kv_base(r, h, 0, br), DH, CT)
        pad = jnp.zeros((256 - DH, SK), kt.dtype)
        kt = jnp.concatenate([kt, pad] if h == 0 else [pad, kt], axis=0)
        return jnp.dot(q, kt, preferred_element_type=jnp.float32)

    def pv(p, r, br, h):
        vt = _slab(u_buf, kv_base(r, h, 1, br), DH, CT)
        return lax.dot_general(vt, p, (((1,), (1,)), ((), ())),
                               preferred_element_type=jnp.float32)

    def qproj(u, br):
        x = _slab(u_buf, X_BASE + (2 * _mod(u, B) + br) * XT, SQ, DT)
        t0 = _div(u, B) * (PW // 128)
        wq = _untile(jnp.stack(
            [wq_buf[br, pl.ds(t0 + rg * QT, PW // 128)] for rg in range(NRG)]))
        q = jnp.dot(x, wq, preferred_element_type=jnp.float32)
        q_sc[_mod(u, QRING), br] = q.astype(jnp.bfloat16)

    def accum(o, u, br):
        row = _mod(u, B) * SQ
        rows = pl.ds(row if isinstance(row, int) else pl.multiple_of(row, SQ), SQ)
        wo = _slab(u_buf, WO_BASE + (2 * _div(u, B) + br) * WOT, PW, DT)
        y = acc_sc[br, rows, :] + jnp.dot(o, wo, preferred_element_type=jnp.float32)
        if not (isinstance(u, int) and u >= NU - B):
            acc_sc[br, rows, :] = y
        out_buf[rows, br * D:(br + 1) * D] = y.astype(out_buf.dtype)

    def body(r, issue):
        sa1 = qk(r, 0, 1)
        issue(0)
        sb1 = qk(r, 1, 1)
        issue(1)
        pa1, la1 = _softmax(sa1)
        sa0 = qk(r, 0, 0)
        issue(2)
        pb1, lb1 = _softmax(sb1)
        oa1 = pv(pa1, r, 0, 1)
        issue(3)
        ob1 = pv(pb1, r, 1, 1)
        issue(4)
        fa = _finish(o0_sc[0], oa1, l0_sc[0], la1)
        qproj(r + QLEAD, 0)
        issue(5)
        pa0, la0 = _softmax(sa0)
        accum(fa, r, 0)
        issue(6)
        sb0 = qk(r, 1, 0)
        issue(7)
        fb = _finish(o0_sc[1], ob1, l0_sc[1], lb1)
        o0_sc[0] = pv(pa0, r, 0, 0)
        l0_sc[0] = la0
        issue(8)
        qproj(r + QLEAD, 1)
        issue(9)
        pb0, lb0 = _softmax(sb0)
        accum(fb, r, 1)
        issue(10)
        o0_sc[1] = pv(pb0, r, 1, 0)
        l0_sc[1] = lb0
        issue(11)

    nq, nsub = len(_QC) - 1, 4
    for i in range(nq // nsub):
        for sub in range(nsub):
            wq_pair(sub * (nq // nsub) + i)
    acc_sc[...] = jnp.zeros_like(acc_sc)
    wq_wait(0)

    first = _merge(x_pairs(range(QLEAD)), kv_half(-1, 0))
    feed = _Feeder(
        first
        + _merge(kv_round(0), [part(wo_pair, 0, p) for p in range(2 * B)],
                 x_pairs(range(QLEAD, B)))
        + _merge(kv_round(1), [part(wo_pair, 1, p) for p in range(2 * (W_LEAD - B))]))
    feed(len(first) + 60)
    wq_wait(1)
    x_wait(0)
    kv_half_wait(-1, 0)
    for u in range(2):
        for br in range(2):
            qproj(u, br)
            feed(4)
    s0 = []
    for br in range(2):
        s0.append(qk(-1, br, 0))
        feed(4)
    for br in range(2):
        for u in range(2, QLEAD):
            qproj(u, br)
            feed(4)
        p0, l0 = _softmax(s0[br])
        o0_sc[br] = pv(p0, -1, br, 0)
        l0_sc[br] = l0
        feed(4)
    feed(len(feed.plan))
    wo_wait(0)
    x_wait(1)

    def step(r, carry):
        gw = _div(r + W_LEAD, B)
        iw = _mod(r + W_LEAD, B)
        plan = kv_round(r + 2)

        def issue(pt):
            for f in plan[4 * pt:4 * pt + 4]:
                f()
            if pt in (3, 9):
                pl.when(gw < NP)(part(wo_pair, gw, 2 * iw + pt // 6))

        pl.when(_mod(r, B) == B - 1)(part(wo_wait, _div(r, B) + 1))
        kv_wait(r)
        body(r, issue)
        return carry

    r0 = NU - QLEAD
    lax.fori_loop(0, r0 - 1, step, 0)

    halves = [(r, h) for r in range(r0 + 1, NU - 1) for h in (1, 0)]
    half_sem = {(r, h): (None if h == 1 else NBUF + r - r0 - 1) for r, h in halves}
    last_sem = NBUF + QLEAD - 2
    r2, r3 = NU - 2, NU - 1
    feed = _Feeder([f for r, h in halves[:-1] for f in kv_half(r, h, half_sem[r, h])]
                   + _merge(kv_half(r2, 0, half_sem[r2, 0]), kv_half(r3, 1, None, (0,)))
                   + kv_half(r3, 1, last_sem, (1,)))
    kv_wait(r0 - 1)
    body(r0 - 1, lambda pt: feed(4))

    kv_wait(r0)
    sa1 = qk(r0, 0, 1)
    feed(4)
    sb1 = qk(r0, 1, 1)
    feed(4)
    pa1, la1 = _softmax(sa1)
    oa1 = pv(pa1, r0, 0, 1)
    feed(4)
    sa0 = qk(r0, 0, 0)
    feed(4)
    pb1, lb1 = _softmax(sb1)
    ob1 = pv(pb1, r0, 1, 1)
    feed(4)
    fa = _finish(o0_sc[0], oa1, l0_sc[0], la1)
    pa0, la0 = _softmax(sa0)
    sb0 = qk(r0, 1, 0)
    feed(4)
    done = {(r0 + 1, 0, 0): (pv(pa0, r0, 0, 0), la0)}
    feed(4)
    ready = [(_finish(o0_sc[1], ob1, l0_sc[1], lb1), r0, 1)]
    prev = _softmax(sb0) + (r0, 0)
    accum(fa, r0, 0)
    feed(4)

    def complete(u, br):
        (o0, l0), (o1, l1) = done[u, br, 0], done[u, br, 1]
        ready.append((_finish(o0, o1, l0, l1), u, br))

    def project():
        accum(*ready.pop(0))

    def prev_pv(p, l, r, h):
        done[r + 1 - h, 1, h] = (pv(p, r, 1, h), l)
        if h == 1:
            complete(r, 1)

    for r, h in halves[:-1]:
        kv_half_wait(r, h, half_sem[r, h])
        sx = qk(r, 0, h)
        feed(4)
        if h == 0:
            complete(r, 0)
        prev_pv(*prev)
        feed(4)
        sy = qk(r, 1, h)
        feed(4)
        px, lx = _softmax(sx)
        if ready:
            project()
        feed(4)
        done[r + 1 - h, 0, h] = (pv(px, r, 0, h), lx)
        feed(4)
        prev = _softmax(sy) + (r, h)
        if (r, h) == halves[-3]:
            project()
            feed(4)
    assert not feed.plan
    complete(r2, 0)
    prev_pv(*prev)
    while ready:
        project()

    kv_half_wait(r2, 0, half_sem[r2, 0])
    kv_half_wait(r3, 1, None, (0,))
    out_start(0)
    s = [qk(r2, 0, 0), qk(r2, 1, 0), qk(r3, 0, 1)]
    pa0, la0 = _softmax(s[0])
    oa0 = pv(pa0, r2, 0, 0)
    kv_half_wait(r3, 1, last_sem, (1,))
    sb1 = qk(r3, 1, 1)
    pb0, lb0 = _softmax(s[1])
    pa1, la1 = _softmax(s[2])
    oa1 = pv(pa1, r3, 0, 1)
    ob0 = pv(pb0, r2, 1, 0)
    pb1, lb1 = _softmax(sb1)
    ob1 = pv(pb1, r3, 1, 1)
    accum(_finish(oa0, oa1, la0, la1), r3, 0)
    out_start(1)
    accum(_finish(ob0, ob1, lb0, lb1), r3, 1)
    out_start(2)
    for i in range(len(out_parts)):
        out_wait(i)


@jax.jit
def pallas_concat_heads__mha_block_cached__gqa_block_cached__near_ridge_kernel(
    A_x: jax.Array,
    A_k_cache: jax.Array,
    A_v_cache: jax.Array,
    A_wq: jax.Array,
    A_wo: jax.Array,
    B_x: jax.Array,
    B_k_cache: jax.Array,
    B_v_cache: jax.Array,
    B_wq: jax.Array,
    B_wo: jax.Array,
):
    for kv in (A_k_cache, A_v_cache, B_k_cache, B_v_cache):
        assert kv.shape == (B, H, SK, DH)

    def tiles(a):
        *lead, rr, cc = a.shape
        a = a.reshape(*lead, rr // 8, 8, cc // 128, 128)
        return jnp.swapaxes(a, -3, -2).reshape(*lead, rr // 8 * (cc // 128), 8, 128)

    def prep(x, k, v, wq, wo):
        return (tiles(x.reshape(B * SQ, D)), tiles(wq), tiles(jnp.swapaxes(k, 2, 3)),
                tiles(jnp.swapaxes(v, 2, 3)), tiles(wo))

    any_spec = pl.BlockSpec(memory_space=pl.ANY)
    out = pl.pallas_call(
        _kernel,
        in_specs=[any_spec] * 10,
        out_specs=any_spec,
        out_shape=jax.ShapeDtypeStruct((B * SQ, 2 * D), jnp.bfloat16),
        scratch_shapes=[
            pltpu.VMEM((U_TILES, 8, 128), jnp.bfloat16),
            pltpu.VMEM((2, WQT, 8, 128), jnp.bfloat16),
            pltpu.VMEM((QRING, 2, SQ, PW), jnp.bfloat16),
            pltpu.VMEM((2, DH, SQ), jnp.float32),
            pltpu.VMEM((2, SQ, 1), jnp.float32),
            pltpu.VMEM((2, B * SQ, D), jnp.float32),
            pltpu.VMEM((B * SQ, 2 * D), jnp.bfloat16),
            pltpu.SemaphoreType.DMA((2,)),
            pltpu.SemaphoreType.DMA((2,)),
            pltpu.SemaphoreType.DMA((2,)),
            pltpu.SemaphoreType.DMA((NBUF + QLEAD - 1,)),
            pltpu.SemaphoreType.DMA((3,)),
        ],
        compiler_params=pltpu.CompilerParams(
            vmem_limit_bytes=100 * 1024 * 1024,
            disable_bounds_checks=True,
            disable_semaphore_checks=True,
        ),
    )(*prep(A_x, A_k_cache, A_v_cache, A_wq, A_wo), *prep(B_x, B_k_cache, B_v_cache, B_wq, B_wo))
    return out.reshape(B, SQ, 2 * D)
```

```python
import functools
import math

import jax
import jax.numpy as jnp
from jax import lax
import jax.experimental.pallas as pl
import jax.experimental.pallas.tpu as pltpu

B, SQ, D, H, SK, DH = 8, 128, 640, 32, 1024, 192
NP = H // 2
PW = 2 * DH
NU = NP * B
SCALE = (DH ** -0.5) * math.log2(math.e)

NBUF = 4
QLEAD = 5
QRING = 8
W_LEAD = 11
OUT_CH = 16
BLK = 16
SHIFT = 13

CT = SK // 128
HT = DH // 8 * CT
DT = D // 128
XT = SQ // 8 * DT
WOT = PW // 8 * DT
QT = H * DH // 128
NRG = D // 8
WQT = NRG * QT


def _cuts(ntiles):
    inner = [SHIFT + BLK * k for k in range(ntiles // BLK) if 0 < SHIFT + BLK * k < ntiles]
    while len(inner) > ntiles // BLK - 1:
        inner = inner[:-1] if SHIFT >= BLK // 2 else inner[1:]
    return [0] + inner + [ntiles]


_KC = _cuts(HT)
_XC = _cuts(XT)
_QC = _cuts(WQT)
_OC = _cuts(WOT)
NCH = len(_KC) - 1

SLOT_T = 4 * 2 * HT
X_BASE = NBUF * SLOT_T
WO_BASE = X_BASE + B * 2 * XT
U_TILES = WO_BASE + NP * 2 * WOT


def _untile(v):
    n, ct = v.shape[:2]
    return jnp.concatenate([v[:, c].reshape(n * 8, 128) for c in range(ct)], axis=1)


def _slab(u_ref, t0, nrows, ct):
    n = nrows // 8
    return _untile(u_ref[pl.ds(t0, n * ct)].reshape(n, ct, 8, 128))


def _softmax(s):
    m = jnp.max(s, axis=-1, keepdims=True)
    p = jnp.exp2((s - m) * SCALE)
    l = jnp.sum(p, axis=-1, keepdims=True)
    return p.astype(jnp.bfloat16), l


def _finish(ot0, ot1, l0, l1):
    o = jnp.concatenate([ot0, ot1], axis=0).T
    lane = lax.broadcasted_iota(jnp.int32, (SQ, PW), 1)
    inv = jnp.where(lane < DH, 1.0 / l0, 1.0 / l1)
    return (o * inv).astype(jnp.bfloat16)


def _div(v, n):
    return v // n if isinstance(v, int) else lax.shift_right_logical(v, n.bit_length() - 1)


def _mod(v, n):
    return v % n if isinstance(v, int) else v & (n - 1)


def _merge(*lists):
    items = [((i + 0.5) / len(l), n, f) for n, l in enumerate(lists) for i, f in enumerate(l)]
    return [f for _, _, f in sorted(items, key=lambda t: t[:2])]


class _Feeder:
    def __init__(self, plan):
        self.plan = list(plan)

    def __call__(self, n):
        now, self.plan = self.plan[:n], self.plan[n:]
        for f in now:
            f()


def _kernel(xa_hbm, wqa_hbm, ka_hbm, va_hbm, woa_hbm,
            xb_hbm, wqb_hbm, kb_hbm, vb_hbm, wob_hbm,
            out_hbm,
            u_buf, wq_buf, q_sc, o0_sc, l0_sc, acc_sc, out_buf,
            sem_x, sem_wq, sem_wo, sem_kv, sem_out):
    x_hbm = (xa_hbm, xb_hbm)
    wq_hbm = (wqa_hbm, wqb_hbm)
    wo_hbm = (woa_hbm, wob_hbm)
    kv_hbm = (ka_hbm, va_hbm, kb_hbm, vb_hbm)
    part = functools.partial

    def wait_all(ref, sem):
        pltpu.make_async_copy(ref, ref, sem).wait()

    def x_pair(b, c):
        t0, nt = _XC[c], _XC[c + 1] - _XC[c]
        for br in range(2):
            pltpu.make_async_copy(x_hbm[br].at[pl.ds(b * XT + t0, nt)],
                                  u_buf.at[pl.ds(X_BASE + (2 * b + br) * XT + t0, nt)],
                                  sem_x.at[0 if b < QLEAD else 1]).start(priority=br)

    def x_pairs(bs):
        return [part(x_pair, b, c) for b in bs for c in range(len(_XC) - 1)]

    def x_wait(i):
        t0, nt = (0, 2 * QLEAD * XT) if i == 0 else (2 * QLEAD * XT, 2 * (B - QLEAD) * XT)
        wait_all(u_buf.at[pl.ds(X_BASE + t0, nt)], sem_x.at[i])

    def wq_pair(c):
        t0, nt = _QC[c], _QC[c + 1] - _QC[c]
        for br in range(2):
            pltpu.make_async_copy(wq_hbm[br].at[pl.ds(t0, nt)], wq_buf.at[br, pl.ds(t0, nt)],
                                  sem_wq.at[min(c, 1)]).start(priority=br)

    def wq_wait(i):
        t0, nt = (0, _QC[1]) if i == 0 else (_QC[1], WQT - _QC[1])
        wait_all(wq_buf.at[:, pl.ds(t0, nt)], sem_wq.at[i])

    def wo_pair(g, t0, nt):
        for br in range(2):
            pltpu.make_async_copy(wo_hbm[br].at[pl.ds(g * WOT + t0, nt)],
                                  u_buf.at[pl.ds(WO_BASE + (2 * g + br) * WOT + t0, nt)],
                                  sem_wo.at[_mod(g, 2)]).start(priority=br)

    def wo_pairs(g, n):
        return [part(wo_pair, g, _OC[c], _OC[c + 1] - _OC[c]) for c in range(n)]

    def wo_pair_dyn(g, c, parity):
        last = len(_OC) - 2
        ok = g < NP
        pl.when(ok & (c > 0) & (c < last))(part(wo_pair, g, _OC[1] + (c - 1) * BLK, BLK))
        for e in (0, last):
            if e % 2 == parity:
                pl.when(ok & (c == e))(part(wo_pair, g, _OC[e], _OC[e + 1] - _OC[e]))

    def wo_wait(g):
        wait_all(u_buf.at[pl.ds(WO_BASE + 2 * g * WOT, 2 * WOT)], sem_wo.at[_mod(g, 2)])

    def slot_of(r):
        return _mod(r + 1, NBUF)

    def kv_base(r, h, kv, br):
        return slot_of(r) * SLOT_T + (4 * h + 2 * kv + br) * HT

    def kv_pair(r, h, c, kv, sem=None):
        u = r + 1 - h
        t0, nt = _KC[c], _KC[c + 1] - _KC[c]
        sem = sem_kv.at[slot_of(r) if sem is None else sem]
        for br in range(2):
            pltpu.make_async_copy(
                kv_hbm[2 * br + kv].at[_mod(u, B), 2 * _div(u, B) + h, pl.ds(t0, nt)],
                u_buf.at[pl.ds(kv_base(r, h, kv, br) + t0, nt)], sem).start(priority=br)

    def kv_round(r):
        return [part(kv_pair, r, h, c, kv) for c in range(NCH) for h in (1, 0) for kv in range(2)]

    def kv_half(r, h, sem=None, kvs=(0, 1)):
        return [part(kv_pair, r, h, c, kv, sem) for c in range(NCH) for kv in kvs]

    def kv_wait(r):
        wait_all(u_buf.at[pl.ds(kv_base(r, 0, 0, 0), SLOT_T)], sem_kv.at[slot_of(r)])

    def kv_half_wait(r, h, sem=None, kvs=(0, 1)):
        wait_all(u_buf.at[pl.ds(kv_base(r, h, kvs[0], 0), 2 * len(kvs) * HT)],
                 sem_kv.at[slot_of(r) if sem is None else sem])

    out_parts = ((0, (B - 1) * SQ, 8, 0, 2 * D),
                 ((B - 1) * SQ, SQ, 4, 0, D), ((B - 1) * SQ, SQ, 4, D, D))

    def out_start(i):
        lo, nrows, ns, c0, nc = out_parts[i]
        n = nrows // OUT_CH
        for k in range(n):
            c = (k % ns) * (n // ns) + k // ns
            rows = pl.ds(lo + c * OUT_CH, OUT_CH)
            pltpu.make_async_copy(out_buf.at[rows, pl.ds(c0, nc)], out_hbm.at[rows, pl.ds(c0, nc)],
                                  sem_out.at[i]).start(priority=k % 2)

    def out_wait(i):
        lo, nrows, _, c0, nc = out_parts[i]
        idx = (pl.ds(lo, nrows), pl.ds(c0, nc))
        pltpu.make_async_copy(out_buf.at[idx], out_hbm.at[idx], sem_out.at[i]).wait()

    def qk(r, br, h):
        q = q_sc[_mod(r + 1 - h, QRING), br, :, h * 128:h * 128 + 256]
        kt = _slab(u_buf, kv_base(r, h, 0, br), DH, CT)
        pad = jnp.zeros((256 - DH, SK), kt.dtype)
        kt = jnp.concatenate([kt, pad] if h == 0 else [pad, kt], axis=0)
        return jnp.dot(q, kt, preferred_element_type=jnp.float32)

    def pv(p, r, br, h):
        vt = _slab(u_buf, kv_base(r, h, 1, br), DH, CT)
        return lax.dot_general(vt, p, (((1,), (1,)), ((), ())),
                               preferred_element_type=jnp.float32)

    def qproj(u, br):
        x = _slab(u_buf, X_BASE + (2 * _mod(u, B) + br) * XT, SQ, DT)
        t0 = _div(u, B) * (PW // 128)
        wq = _untile(jnp.stack(
            [wq_buf[br, pl.ds(t0 + rg * QT, PW // 128)] for rg in range(NRG)]))
        q = jnp.dot(x, wq, preferred_element_type=jnp.float32)
        q_sc[_mod(u, QRING), br] = q.astype(jnp.bfloat16)

    def accum(o, u, br):
        row = _mod(u, B) * SQ
        rows = pl.ds(row if isinstance(row, int) else pl.multiple_of(row, SQ), SQ)
        wo = _slab(u_buf, WO_BASE + (2 * _div(u, B) + br) * WOT, PW, DT)
        y = acc_sc[br, rows, :] + jnp.dot(o, wo, preferred_element_type=jnp.float32)
        if not (isinstance(u, int) and u >= NU - B):
            acc_sc[br, rows, :] = y
        out_buf[rows, br * D:(br + 1) * D] = y.astype(out_buf.dtype)

    def body(r, issue):
        sa1 = qk(r, 0, 1)
        issue(0)
        sb1 = qk(r, 1, 1)
        issue(1)
        pa1, la1 = _softmax(sa1)
        sa0 = qk(r, 0, 0)
        issue(2)
        pb1, lb1 = _softmax(sb1)
        oa1 = pv(pa1, r, 0, 1)
        issue(3)
        ob1 = pv(pb1, r, 1, 1)
        issue(4)
        fa = _finish(o0_sc[0], oa1, l0_sc[0], la1)
        qproj(r + QLEAD, 0)
        issue(5)
        pa0, la0 = _softmax(sa0)
        accum(fa, r, 0)
        issue(6)
        sb0 = qk(r, 1, 0)
        issue(7)
        fb = _finish(o0_sc[1], ob1, l0_sc[1], lb1)
        o0_sc[0] = pv(pa0, r, 0, 0)
        l0_sc[0] = la0
        issue(8)
        qproj(r + QLEAD, 1)
        issue(9)
        pb0, lb0 = _softmax(sb0)
        accum(fb, r, 1)
        issue(10)
        o0_sc[1] = pv(pb0, r, 1, 0)
        l0_sc[1] = lb0
        issue(11)

    nq, nsub = len(_QC) - 1, 4
    for i in range(nq // nsub):
        for sub in range(nsub):
            wq_pair(sub * (nq // nsub) + i)
    acc_sc[...] = jnp.zeros_like(acc_sc)
    wq_wait(0)

    first = _merge(x_pairs(range(QLEAD)), kv_half(-1, 0))
    feed = _Feeder(
        first
        + _merge(kv_round(0), wo_pairs(0, len(_OC) - 1), x_pairs(range(QLEAD, B)))
        + _merge(kv_round(1), wo_pairs(1, 2 * (W_LEAD - B))))
    feed(len(first) + 60)
    wq_wait(1)
    x_wait(0)
    kv_half_wait(-1, 0)
    for u in range(2):
        for br in range(2):
            qproj(u, br)
            feed(4)
    s0 = []
    for br in range(2):
        s0.append(qk(-1, br, 0))
        feed(4)
    for br in range(2):
        for u in range(2, QLEAD):
            qproj(u, br)
            feed(4)
        p0, l0 = _softmax(s0[br])
        o0_sc[br] = pv(p0, -1, br, 0)
        l0_sc[br] = l0
        feed(4)
    feed(len(feed.plan))
    wo_wait(0)
    x_wait(1)

    def step(r, carry):
        gw = _div(r + W_LEAD, B)
        iw = _mod(r + W_LEAD, B)
        plan = kv_round(r + 2)

        def issue(pt):
            for f in plan[4 * pt:4 * pt + 4]:
                f()
            if pt in (3, 9):
                wo_pair_dyn(gw, 2 * iw + pt // 6, pt // 6)

        pl.when(_mod(r, B) == B - 1)(part(wo_wait, _div(r, B) + 1))
        kv_wait(r)
        body(r, issue)
        return carry

    r0 = NU - QLEAD
    lax.fori_loop(0, r0 - 1, step, 0)

    halves = [(r, h) for r in range(r0 + 1, NU - 1) for h in (1, 0)]
    half_sem = {(r, h): (None if h == 1 else NBUF + r - r0 - 1) for r, h in halves}
    last_sem = NBUF + QLEAD - 2
    r2, r3 = NU - 2, NU - 1
    feed = _Feeder([f for r, h in halves[:-1] for f in kv_half(r, h, half_sem[r, h])]
                   + _merge(kv_half(r2, 0, half_sem[r2, 0]), kv_half(r3, 1, None, (0,)))
                   + kv_half(r3, 1, last_sem, (1,)))
    kv_wait(r0 - 1)
    body(r0 - 1, lambda pt: feed(4))

    kv_wait(r0)
    sa1 = qk(r0, 0, 1)
    feed(4)
    sb1 = qk(r0, 1, 1)
    feed(4)
    pa1, la1 = _softmax(sa1)
    oa1 = pv(pa1, r0, 0, 1)
    feed(4)
    sa0 = qk(r0, 0, 0)
    feed(4)
    pb1, lb1 = _softmax(sb1)
    ob1 = pv(pb1, r0, 1, 1)
    feed(4)
    fa = _finish(o0_sc[0], oa1, l0_sc[0], la1)
    pa0, la0 = _softmax(sa0)
    sb0 = qk(r0, 1, 0)
    feed(4)
    done = {(r0 + 1, 0, 0): (pv(pa0, r0, 0, 0), la0)}
    feed(4)
    ready = [(_finish(o0_sc[1], ob1, l0_sc[1], lb1), r0, 1)]
    prev = _softmax(sb0) + (r0, 0)
    accum(fa, r0, 0)
    feed(4)

    def complete(u, br):
        (o0, l0), (o1, l1) = done[u, br, 0], done[u, br, 1]
        ready.append((_finish(o0, o1, l0, l1), u, br))

    def project():
        accum(*ready.pop(0))

    def prev_pv(p, l, r, h):
        done[r + 1 - h, 1, h] = (pv(p, r, 1, h), l)
        if h == 1:
            complete(r, 1)

    for r, h in halves[:-1]:
        kv_half_wait(r, h, half_sem[r, h])
        sx = qk(r, 0, h)
        feed(4)
        if h == 0:
            complete(r, 0)
        prev_pv(*prev)
        feed(4)
        sy = qk(r, 1, h)
        feed(4)
        px, lx = _softmax(sx)
        if ready:
            project()
        feed(4)
        done[r + 1 - h, 0, h] = (pv(px, r, 0, h), lx)
        feed(4)
        prev = _softmax(sy) + (r, h)
        if (r, h) == halves[-3]:
            project()
            feed(4)
    assert not feed.plan
    complete(r2, 0)
    prev_pv(*prev)
    while ready:
        project()

    kv_half_wait(r2, 0, half_sem[r2, 0])
    kv_half_wait(r3, 1, None, (0,))
    out_start(0)
    s = [qk(r2, 0, 0), qk(r2, 1, 0), qk(r3, 0, 1)]
    pa0, la0 = _softmax(s[0])
    oa0 = pv(pa0, r2, 0, 0)
    kv_half_wait(r3, 1, last_sem, (1,))
    sb1 = qk(r3, 1, 1)
    pb0, lb0 = _softmax(s[1])
    pa1, la1 = _softmax(s[2])
    oa1 = pv(pa1, r3, 0, 1)
    ob0 = pv(pb0, r2, 1, 0)
    pb1, lb1 = _softmax(sb1)
    ob1 = pv(pb1, r3, 1, 1)
    accum(_finish(oa0, oa1, la0, la1), r3, 0)
    out_start(1)
    accum(_finish(ob0, ob1, lb0, lb1), r3, 1)
    out_start(2)
    for i in range(len(out_parts)):
        out_wait(i)


@jax.jit
def pallas_concat_heads__mha_block_cached__gqa_block_cached__near_ridge_kernel(
    A_x: jax.Array,
    A_k_cache: jax.Array,
    A_v_cache: jax.Array,
    A_wq: jax.Array,
    A_wo: jax.Array,
    B_x: jax.Array,
    B_k_cache: jax.Array,
    B_v_cache: jax.Array,
    B_wq: jax.Array,
    B_wo: jax.Array,
):
    for kv in (A_k_cache, A_v_cache, B_k_cache, B_v_cache):
        assert kv.shape == (B, H, SK, DH)

    def tiles(a):
        *lead, rr, cc = a.shape
        a = a.reshape(*lead, rr // 8, 8, cc // 128, 128)
        return jnp.swapaxes(a, -3, -2).reshape(*lead, rr // 8 * (cc // 128), 8, 128)

    def prep(x, k, v, wq, wo):
        return (tiles(x.reshape(B * SQ, D)), tiles(wq), tiles(jnp.swapaxes(k, 2, 3)),
                tiles(jnp.swapaxes(v, 2, 3)), tiles(wo))

    any_spec = pl.BlockSpec(memory_space=pl.ANY)
    out = pl.pallas_call(
        _kernel,
        in_specs=[any_spec] * 10,
        out_specs=any_spec,
        out_shape=jax.ShapeDtypeStruct((B * SQ, 2 * D), jnp.bfloat16),
        scratch_shapes=[
            pltpu.VMEM((U_TILES, 8, 128), jnp.bfloat16),
            pltpu.VMEM((2, WQT, 8, 128), jnp.bfloat16),
            pltpu.VMEM((QRING, 2, SQ, PW), jnp.bfloat16),
            pltpu.VMEM((2, DH, SQ), jnp.float32),
            pltpu.VMEM((2, SQ, 1), jnp.float32),
            pltpu.VMEM((2, B * SQ, D), jnp.float32),
            pltpu.VMEM((B * SQ, 2 * D), jnp.bfloat16),
            pltpu.SemaphoreType.DMA((2,)),
            pltpu.SemaphoreType.DMA((2,)),
            pltpu.SemaphoreType.DMA((2,)),
            pltpu.SemaphoreType.DMA((NBUF + QLEAD - 1,)),
            pltpu.SemaphoreType.DMA((3,)),
        ],
        compiler_params=pltpu.CompilerParams(
            vmem_limit_bytes=100 * 1024 * 1024,
            disable_bounds_checks=True,
            disable_semaphore_checks=True,
        ),
    )(*prep(A_x, A_k_cache, A_v_cache, A_wq, A_wo), *prep(B_x, B_k_cache, B_v_cache, B_wq, B_wo))
    return out.reshape(B, SQ, 2 * D)
```
